```python
import os as _os
_os.environ.setdefault("JAX_PLATFORMS", "cpu")
import jax
import jax.numpy as jnp

def _softmax(x, axis=-1):
    return jax.nn.softmax(x, axis=axis)
def _gelu(x):
    return jax.nn.gelu(x, approximate=True)
def _silu(x):
    return jax.nn.silu(x)
def _sigmoid(x):
    return jax.nn.sigmoid(x)
def _layernorm(x, axis=-1, eps=1e-5):
    m = jnp.mean(x, axis=axis, keepdims=True)
    v = jnp.var(x, axis=axis, keepdims=True)
    return (x - m) / jnp.sqrt(v + eps)
def _scatter_add(tgt, idx, src, axis=0):
    return tgt.at[idx].add(src)
def _segment_sum(src, seg, n):
    return jax.ops.segment_sum(src, seg, n)
class _Rng:
    def __init__(self, key):
        self._k = key
    def _next(self):
        self._k, sub = jax.random.split(self._k)
        return sub
    def normal(self, shape):
        return jax.random.normal(self._next(), shape, dtype=jnp.bfloat16)
    def randint(self, lo, hi, shape):
        return jax.random.randint(self._next(), shape, lo, hi, dtype=jnp.int32)
    def uniform(self, shape, lo=0.0, hi=1.0):
        return jax.random.uniform(self._next(), shape, jnp.bfloat16, lo, hi)
    def permutation(self, n):
        return jax.random.permutation(self._next(), n)


kernel_name = 'concat_heads__grouped_kv_mqa__sliding_block__prompt'

def setup_inputs():
    _rng = _Rng(jax.random.key(int.from_bytes(__import__("os").urandom(4), "little")))
    _w = (lambda a: (lambda t: t.astype(jnp.bfloat16) if jnp.issubdtype(t.dtype, jnp.floating) else t)(jnp.asarray(a)))
    def _A_setup():
        B, S, D, H = 1, 2048, 576, 32
        Dh = D // H
        return {
            "x": _w((lambda *s: _rng.normal(s) * 0.05)(B, S, D)),
            "wq": _w((lambda *s: _rng.normal(s) * 1.6)(D, H * Dh)),
            "wk": _w((lambda *s: _rng.normal(s) * 1.6)(D, Dh)),
            "wv": _w((lambda *s: _rng.normal(s) * 0.1)(D, Dh)),
            "wo": _w((lambda *s: _rng.normal(s) * 0.1)(H * Dh, D)),
        }
    _A_in = _A_setup()

    def _B_setup():
        B, S, D = 1, 2048, 576
        return {
            "x": _w((lambda *s: _rng.normal(s) * 0.2)(B, S, D)),
            "wqkv": _w((lambda *s: _rng.normal(s) * 0.2)(D, 3 * D)),
            "wo": _w((lambda *s: _rng.normal(s) * 0.05)(D, D)),
        }
    _B_in = _B_setup()

    return {
        "A_x": _A_in["x"],
        "A_wq": _A_in["wq"],
        "A_wk": _A_in["wk"],
        "A_wv": _A_in["wv"],
        "A_wo": _A_in["wo"],
        "B_x": _B_in["x"],
        "B_wqkv": _B_in["wqkv"],
        "B_wo": _B_in["wo"],
    }

def reference(A_x, A_wq, A_wk, A_wv, A_wo, B_x, B_wqkv, B_wo):
    def _A_ref(x, wq, wk, wv, wo):
        B, S, D = x.shape
        H = 32
        Dh = D // H
        q = (lambda x, *d: x.transpose(*d))((x @ wq).reshape(B, S, H, Dh), 0, 2, 1, 3)
        k = x @ wk
        v = x @ wv
        scores = jnp.einsum("bhqd,bkd->bhqk", q, k) * (Dh ** -0.5)
        p = _softmax(scores, axis=-1)
        o = jnp.einsum("bhqk,bkd->bhqd", p, v)
        return (lambda x, *d: x.transpose(*d))(o, 0, 2, 1, 3).reshape(B, S, H * Dh) @ wo

    def _B_ref(x, wqkv, wo):
        B, S, D = x.shape
        H = 32; Dh = D // H; W = 256
        qkv = (lambda x, *d: x.transpose(*d))((x @ wqkv).reshape(B, S, 3, H, Dh), 2, 0, 3, 1, 4)
        q, k, v = qkv[0], qkv[1], qkv[2]
        scores = jnp.einsum("bhqd,bhkd->bhqk", q, k) * (Dh ** -0.5)
        idx = jnp.arange(S)
        mask = (idx[:, None] - idx[None, :] >= 0) & (idx[:, None] - idx[None, :] < W)
        scores = jnp.where(mask[None, None], scores, -1e9)
        p = _softmax(scores, axis=-1)
        o = jnp.einsum("bhqk,bhkd->bhqd", p, v)
        return (lambda x, *d: x.transpose(*d))(o, 0, 2, 1, 3).reshape(B, S, D) @ wo

    a = _A_ref(A_x, A_wq, A_wk, A_wv, A_wo)
    b = _B_ref(B_x, B_wqkv, B_wo)
    return jnp.concatenate([a, b], axis=-1)
```

```python
import functools

import jax
import jax.numpy as jnp
import numpy as np
from jax import lax
import jax.experimental.pallas as pl
import jax.experimental.pallas.tpu as pltpu

f32, bf16, u32, i32 = jnp.float32, jnp.bfloat16, jnp.uint32, jnp.int32

S = 2048
D = 576
H = 32
DH = 18
WIN = 256
NQ = 512
NB = S // NQ
CK = 128
NC = S // CK
HR = 24
HPT = 7
NT = -(-H // HPT)
QSCALE = float(DH ** -0.5 * np.log2(np.e))
L_MIN = float(2.0 ** -50)
NEG = -1e30

JA = 2
JB = 2


def _dot(a, b):
    return lax.dot_general(a, b, (((1,), (0,)), ((), ())), preferred_element_type=f32)


def _pack(x):
    return pltpu.bitcast(x, u32)


def _unpack(x):
    return pltpu.bitcast(x, bf16)


def _round(x):
    return x.astype(bf16).astype(f32)


def _iota(shape, axis):
    return lax.broadcasted_iota(i32, shape, axis)


def _kernel(xa_h, wqa_h, wka_h, wva_h, woa_h, xb_h, wqkv_h, wob_h, out_h,
            xa, xb, wqa, wka, wva, woa, wqkv, wob,
            wt, qa, kta, ka, vta, pa, op,
            qb, ktb, kb, vtb, sb, mb, umask, obt, outv, sems, osems):
    def xcopy(src, dst, nb, sem):
        return pltpu.make_async_copy(src.at[:, nb * NQ:(nb + 1) * NQ], dst.at[:, nb * NQ:(nb + 1) * NQ], sems.at[sem])

    c_wqa = pltpu.make_async_copy(wqa_h, wqa, sems.at[0])
    c_wka = pltpu.make_async_copy(wka_h, wka, sems.at[1])
    c_wva = pltpu.make_async_copy(wva_h, wva, sems.at[2])
    c_xa = [xcopy(xa_h, xa, nb, 3 + nb) for nb in range(NB)]
    c_wqkv = pltpu.make_async_copy(wqkv_h, wqkv, sems.at[7])
    c_xb = pltpu.make_async_copy(xb_h, xb, sems.at[8])
    c_wob = pltpu.make_async_copy(wob_h, wob, sems.at[9])
    c_woa = pltpu.make_async_copy(woa_h, woa, sems.at[10])
    for c in [c_wqa, c_wka, c_wva] + c_xa + [c_wqkv, c_xb, c_wob, c_woa]:
        c.start()

    row8 = _iota((8, NQ), 0)

    c_wqa.wait()
    wt[0:D // 2, :] = _pack(wqa[...].T)
    c_wka.wait()
    c_wva.wait()
    z6 = jnp.zeros((HR - DH, D), f32)
    wkv = jnp.concatenate([wka[...].astype(f32), z6, wva[...].astype(f32), z6], axis=0)
    wt[D // 2:D // 2 + HR, :] = _pack(wkv.astype(bf16))
    for nb in range(NB):
        c_xa[nb].wait()
        cols = slice(nb * NQ, (nb + 1) * NQ)
        y = _dot(_unpack(wt[0:D // 2 + HR, :]), xa[:, cols])
        kta[:, cols] = _round(y[D:D + HR])
        v = _round(y[D + HR:D + 2 * HR])
        vta[0:16, cols] = v[0:16]
        vta[16:HR, cols] = jnp.where(row8 == DH - 16, 1.0, v[16:HR])
        ys = y * QSCALE
        for h in range(H):
            q = ys[h * DH:h * DH + HR]
            q2 = jnp.where(row8 < DH - 16, q[16:HR], 0.0)
            nrm = jnp.sum(q[0:8] * q[0:8] + q[8:16] * q[8:16] + q2 * q2, axis=0, keepdims=True)
            nrm = jnp.sqrt(nrm) * -1.02
            q2 = jnp.where(row8 == DH - 16, nrm, q2)
            qh = jnp.concatenate([q[0:16], q2, jnp.zeros((8, NQ), f32)], axis=0)
            qa[nb * H + h] = _pack(qh.astype(bf16))
    kt = kta[...]
    kmax = jnp.sqrt(jnp.max(jnp.sum(kt * kt, axis=0, keepdims=True), axis=1, keepdims=True)) * 1.02
    kt = jnp.concatenate([kt[0:16], jnp.where(_iota((8, S), 0) == DH - 16, kmax, kt[16:HR]),
                          jnp.zeros((128 - HR, S), f32)], axis=0)
    ka[...] = _pack(kt.astype(bf16).T)

    c_wqkv.wait()
    wt[...] = _pack(wqkv[...].T)
    c_xb.wait()

    def b_proj(nb, _):
        cols = pl.ds(pl.multiple_of(nb * NQ, NQ), NQ)
        y = _dot(_unpack(wt[...]), xb[:, cols])
        q = _pack((y[0:D] * QSCALE).astype(bf16))
        k = _pack(y[D:2 * D].astype(bf16))
        pad = jnp.zeros((64, NQ), u32)
        q = jnp.concatenate([q, pad], axis=0)
        k = jnp.concatenate([k, pad], axis=0)
        for t in range(NT):
            r0 = t * HPT * DH // 2
            qb[t, :, cols] = q[r0:r0 + 64]
            kb[t, pl.ds(pl.multiple_of(nb * (NQ // 2), NQ // 2), NQ // 2), :] = _pack(_unpack(k[r0:r0 + 64]).T)
        v = _round(y[2 * D:3 * D])
        v = jnp.concatenate([v, jnp.zeros((8, NQ), f32)], axis=0)
        for h in range(H):
            vh = v[h * DH:h * DH + HR]
            vtb[h, 0:16, cols] = vh[0:16]
            vtb[h, 16:HR, cols] = jnp.where(row8 < DH - 16, vh[16:HR], jnp.where(row8 == DH - 16, 1.0, 0.0))
        return None

    lax.fori_loop(0, NB, b_proj, None)

    upper = _iota((CK, CK), 0) > _iota((CK, CK), 1)
    umask[...] = _pack(jnp.where(upper, -1.0, 0.0).astype(bf16)) | jnp.uint32(0)
    um = umask[...]
    umask[...] = (jnp.where((um & jnp.uint32(0xFFFF)) != 0, jnp.uint32(0xFFFF), jnp.uint32(0))
                  | jnp.where((um >> 16) != 0, jnp.uint32(0xFFFF0000), jnp.uint32(0)))

    def b_scores(h, j, t):
        tile = h // HPT
        r0 = (h - tile * HPT) * (DH // 2)
        rr = _iota((64, CK), 0)
        w = _unpack(jnp.where((rr >= r0) & (rr < r0 + DH // 2), qb[tile, :, t * CK:(t + 1) * CK], jnp.uint32(0)))
        k0 = max(0, t - 2)
        s = _dot(_unpack(kb[tile, k0 * CK // 2:(t + 1) * CK // 2, :]), w)
        if t >= 2:
            s = jnp.concatenate([jnp.where(upper, s[0:CK], s[2 * CK:]), s[CK:2 * CK]], axis=0)
        elif t == 1:
            s = jnp.concatenate([jnp.where(upper, NEG, s[CK:]), s[0:CK]], axis=0)
        else:
            s = jnp.where(upper, NEG, s)
        n = s.shape[0]
        sb[j, t, 0:n, :] = s
        m = jnp.max(s.reshape(n // 8, 8, CK), axis=0)
        mb[j, :, t * CK:(t + 1) * CK] = jnp.broadcast_to(jnp.max(m, axis=0, keepdims=True), (8, CK))

    def b_pv(h, j, t):
        n = 2 * CK if t >= 1 else CK
        s = sb[j, t, 0:n, :]
        m = mb[j, :, t * CK:(t + 1) * CK]
        p = _pack(jnp.exp2(s.reshape(n // 8, 8, CK) - m[None]).reshape(n, CK).astype(bf16))
        if t >= 2:
            first = p[0:CK // 2] & umask[...]
            p = jnp.concatenate([first, p[CK // 2:], p[0:CK // 2] ^ first], axis=0)
        elif t == 1:
            p = jnp.concatenate([p[CK // 2:], p[0:CK // 2]], axis=0)
        k0 = max(0, t - 2)
        op[h, :, t * CK:(t + 1) * CK] = _dot(vtb[h, :, k0 * CK:(t + 1) * CK], _unpack(p))

    for j in range(JB):
        for t in range(NC):
            b_scores(j, j, t)

    def b_body(i, _):
        for j in range(JB):
            for t in range(NC):
                b_pv(i * JB + j, j, t)
                b_scores((i + 1) * JB + j, j, t)
        return None

    lax.fori_loop(0, H // JB - 1, b_body, None)
    for j in range(JB):
        for t in range(NC):
            b_pv(H - JB + j, j, t)

    def out_proj(cols):
        o = []
        for h in range(H):
            oh = op[h, :, cols]
            o.append(oh[0:DH] * (1.0 / oh[DH:DH + 1]))
        o = jnp.concatenate(o, axis=0).astype(bf16)
        return _dot(_unpack(wt[0:D // 2, :]), o).astype(bf16)

    c_wob.wait()
    wt[0:D // 2, :] = _pack(wob[...].T)

    def b_out(nb, _):
        cols = pl.ds(pl.multiple_of(nb * NQ, NQ), NQ)
        y = _pack(out_proj(cols))
        obt[:, cols] = y[0:32]
        outv[cols, 640:2 * D] = _unpack(y[32:]).T
        return None

    lax.fori_loop(0, NB, b_out, None)
    c_woa.wait()
    wt[0:D // 2, :] = _pack(woa[...].T)

    def a_probs(w, j, c):
        k = _unpack(ka[c * CK // 2:(c + 1) * CK // 2, :])[:, 0:32]
        pa[j, c * CK // 2:(c + 1) * CK // 2, :] = _pack(jnp.exp2(_dot(k, w)).astype(bf16))

    def a_pv(j, c, acc):
        r = _dot(vta[:, c * CK:(c + 1) * CK], _unpack(pa[j, c * CK // 2:(c + 1) * CK // 2, :]))
        return r if acc is None else acc + r

    def a_step(u, nxt):
        for j in range(JA):
            w = _unpack(qa[u + JA + j]) if nxt else None
            acc = None
            for c in range(NC):
                acc = a_pv(j, c, acc)
                if nxt:
                    a_probs(w, j, c)
            op[(u + j) % H, :, 0:NQ] = acc

    def a_exact(nb):
        def body(h, _):
            w = _unpack(jnp.where(_iota((16, NQ), 0) < DH // 2, qa[nb * H + h], jnp.uint32(0)))
            s = _dot(_unpack(ka[...])[:, 0:32], w)
            p = jnp.exp2(s - jnp.max(s, axis=0, keepdims=True)).astype(bf16)
            op[h, :, 0:NQ] = _dot(vta[...], p)
            return None
        lax.fori_loop(0, H, body, None)

    def out_copy(nb):
        rows = pl.ds(pl.multiple_of(nb * NQ, NQ), NQ)
        return pltpu.make_async_copy(outv.at[rows, :], out_h.at[rows, :], osems.at[nb])

    for j in range(JA):
        w = _unpack(qa[j])
        for c in range(NC):
            a_probs(w, j, c)

    def a_block(nb, _):
        last = nb == NB - 1

        def body(i, _):
            a_step(nb * H + i * JA, True)
            return None

        lax.fori_loop(0, jnp.where(last, H // JA - 1, H // JA), body, None)

        @pl.when(last)
        def _():
            a_step(NB * H - JA, False)

        lmin = op[0, 16:HR, 0:NQ]
        for h in range(1, H):
            lmin = jnp.minimum(lmin, op[h, 16:HR, 0:NQ])
        lmin = jnp.min(jnp.where(row8 == DH - 16, lmin, 1.0))

        @pl.when(jnp.logical_not(lmin >= L_MIN))
        def _():
            a_exact(nb)

        cols = pl.ds(pl.multiple_of(nb * NQ, NQ), NQ)
        y = jnp.concatenate([_pack(out_proj(slice(0, NQ))), obt[:, cols]], axis=0)
        outv[cols, 0:640] = _unpack(y).T
        out_copy(nb).start()
        return None

    lax.fori_loop(0, NB, a_block, None)
    for nb in range(NB):
        out_copy(nb).wait()


@jax.jit
def pallas_concat_heads__grouped_kv_mqa__sliding_block__prompt_kernel(
    A_x: jax.Array,
    A_wq: jax.Array,
    A_wk: jax.Array,
    A_wv: jax.Array,
    A_wo: jax.Array,
    B_x: jax.Array,
    B_wqkv: jax.Array,
    B_wo: jax.Array,
):
    vmem = pltpu.VMEM
    hbm = pl.BlockSpec(memory_space=pltpu.HBM)
    out = pl.pallas_call(
        _kernel,
        out_shape=jax.ShapeDtypeStruct((S, 2 * D), bf16),
        in_specs=[hbm] * 8,
        out_specs=hbm,
        scratch_shapes=[
            vmem((D, S), bf16), vmem((D, S), bf16),
            vmem((D, D), bf16), vmem((DH, D), bf16), vmem((DH, D), bf16), vmem((D, D), bf16),
            vmem((D, 3 * D), bf16), vmem((D, D), bf16),
            vmem((3 * D // 2, D), u32),
            vmem((NB * H, 16, NQ), u32),
            vmem((HR, S), f32),
            vmem((S // 2, 128), u32),
            vmem((HR, S), f32),
            vmem((JA, S // 2, NQ), u32),
            vmem((H, HR, S), f32),
            vmem((NT, 64, S), u32),
            vmem((8, 128), u32),
            vmem((NT, S // 2, 128), u32),
            vmem((H, HR, S), f32),
            vmem((JB, NC, 2 * CK, CK), f32),
            vmem((JB, 8, S), f32),
            vmem((CK // 2, CK), u32),
            vmem((32, S), u32),
            vmem((S, 2 * D), bf16),
            pltpu.SemaphoreType.DMA((11,)),
            pltpu.SemaphoreType.DMA((NB,)),
        ],
        compiler_params=pltpu.CompilerParams(vmem_limit_bytes=110 * 2 ** 20),
        name="attn_pair",
    )(A_x.reshape(S, D).T, A_wq, A_wk.T, A_wv.T, A_wo, B_x.reshape(S, D).T, B_wqkv, B_wo)
    return out.reshape(1, S, 2 * D)
```

```python
import jax
import jax.numpy as jnp
import numpy as np
from jax import lax
import jax.experimental.pallas as pl
import jax.experimental.pallas.tpu as pltpu

f32, bf16, u32, i32 = jnp.float32, jnp.bfloat16, jnp.uint32, jnp.int32

S = 2048
D = 576
H = 32
DH = 18
T = 128
NT = S // T
QT = 4
NQ = QT * T
NB = S // NQ
NU = NB * H
HR = 24
HPT = 4
BU = 32
QSCALE = float(DH ** -0.5 * np.log2(np.e))
SLACK = 1.02
L_MIN = float(2.0 ** -50)
NEG = -1e30

JA = 8
NVS = [32] * 5 + [16] * 11
NFS = [0] * 15 + [16]
QR = DH + 3
SKEW = 1
MC = 96
KS = [0, 128, 256, D]
EARLY = 2
PG = -(-D // T) * D // 16
LEAD = 40


def _dot(a, b):
    return lax.dot_general(a, b, (((1,), (0,)), ((), ())), preferred_element_type=f32)


def _pack(x):
    return pltpu.bitcast(x, u32)


def _unpack(x):
    return pltpu.bitcast(x, bf16)


def _round(x):
    return x.astype(bf16).astype(f32)


def _iota(shape, axis):
    return lax.broadcasted_iota(i32, shape, axis)


def _tile(y, t):
    return y[:, t * T:(t + 1) * T]


def _untile(y):
    return jnp.concatenate([y[t] for t in range(QT)], axis=1)


class _Side:
    def __init__(self):
        self.jobs, self.due, self.clock, self.token = [], [], 0, None

    def add(self, gen, steps, ticks, ahead=0):
        next(gen)
        self.jobs.append(dict(gen=gen, steps=steps, ticks=ticks, ahead=ahead, done=0, seen=0))

    def _run(self, job, upto):
        while job["done"] < min(job["steps"], upto):
            try:
                job["gen"].send(self.token if job["done"] >= job["ahead"] else jnp.zeros((8, T), f32))
            except StopIteration:
                pass
            job["done"] += 1

    def rows(self, y):
        for r in range(0, y.shape[0], 16):
            self.clock += 1
            self.token = y[r + 8:r + 16, y.shape[1] - T:]
            for job in self.jobs:
                job["seen"] += 1
                self._run(job, job["ahead"] - (-job["seen"] * job["steps"] // job["ticks"]))

    def done(self, val):
        self.due.append((self.clock + LEAD, val))

    def take(self):
        ready = [v for t, v in self.due if t <= self.clock]
        self.due = [(t, v) for t, v in self.due if t > self.clock]
        return ready

    def flush(self):
        for job in self.jobs:
            self._run(job, job["steps"])
        self.jobs, self.due = [], []


def _spread(gen, steps, calls):
    next(gen)
    counts = iter([(n + 1) * steps // calls - n * steps // calls for n in range(calls)])

    def call():
        for _ in range(next(counts)):
            next(gen, None)

    return call


def _kernel(xa_h, wqa_h, wka_h, wva_h, woa_h, xb_h, wqkv_h, wob_h, out_h,
            xa, xb, wqa, wka, wva, woa, wqkv, wob, wta, wtb, wtoa, wtob,
            qa, ka, vta, kbc, qbc, pa, pv, pf,
            qb, ktb, kb, kr, vtb, sb, mb, umask,
            ot, obt, outv, order, tmp, sems, osems):
    voff = [int(x) for x in np.cumsum([0] + NVS)]
    foff = [int(x) for x in np.cumsum([0] + NFS)]
    nv, nf = voff[-1], foff[-1]
    row = _iota((8, T), 0)
    zero = jnp.zeros((8, T), f32)
    side = _Side()

    def blk(nb):
        return slice(nb * NQ, (nb + 1) * NQ)

    def dblk(start, size):
        return pl.ds(pl.multiple_of(start, size), size)

    def after(val, tok, i):
        at = (slice(i, i + val.shape[0]), slice(0, val.shape[1])) if val.ndim == 4 else (i, 0)
        order[at] = jnp.broadcast_to(tok, val.shape)
        order[at] = val
        return order[at]

    def paced(lhs):
        ready = side.take()
        if not ready:
            return lhs
        top = pltpu.bitcast(lhs[0:8], f32)
        for tok in ready:
            top = after(top, tok, 0)
        return jnp.concatenate([_pack(top), lhs[8:]], axis=0)

    def packed(e, r0):
        at = (slice(r0, r0 + e.shape[0] // 2), slice(0, e.shape[1]))
        tmp[at] = _pack(e.astype(bf16))
        return tmp[at]

    def proj(w_ref, r0, r1, x, between=None):
        y = None
        for k0 in range(0, D, T):
            k1 = min(k0 + T, D)
            if between is not None:
                between()
            w = w_ref[r0 // 2:r1 // 2, k0:k1]
            part = _dot(_unpack(paced(w) if k1 - k0 == T else w), x[k0:k1])
            side.rows(part)
            y = part if y is None else y + part
        return y

    def write_out(y, r0, c0):
        def tiles():
            for t in range(QT):
                tok = yield
                yt = _tile(y, t)
                yt = jnp.concatenate([after(yt[0:8], tok, 1), yt[8:]], axis=0).astype(bf16).T
                r = r0 + t * T
                outv[slice(r, r + T) if isinstance(r, int) else dblk(r, T), c0:c0 + T] = yt
                side.done(yt[T - 16:T].astype(f32)[8:16])

        side.add(tiles(), QT, 20)

    def put_head(t, h, o):
        den = o[DH:DH + 1]
        inv = pl.reciprocal(den, approx=True)
        ot[t, pl.ds(h * DH, DH), :] = (o * (inv * (2.0 - den * inv)))[0:DH]

    slabs = [slice(a, b) for a, b in zip(KS[:-1], KS[1:])]
    pairs = [(src.at[k, cols], dst.at[k, cols]) for k in slabs
             for src, dst, cols in ((wqa_h, wqa, slice(None)), (xa_h, xa, blk(0)))]
    pairs += [(xa_h.at[:, blk(nb)], xa.at[:, blk(nb)]) for nb in range(1, NB)]
    pairs += [(wka_h, wka), (wva_h, wva), (wqkv_h, wqkv), (wob_h, wob), (woa_h, woa)]
    copies = [pltpu.make_async_copy(src, dst, sems.at[n]) for n, (src, dst) in enumerate(pairs)]
    c_slab = [copies[2 * n:2 * n + 2] for n in range(len(slabs))]
    c_xa1, c_xa2, c_xa3, c_wka, c_wva, c_wqkv, c_wob, c_woa = copies[2 * len(slabs):]

    def c_xb(nb):
        cols = blk(nb) if isinstance(nb, int) else dblk(nb * NQ, NQ)
        return pltpu.make_async_copy(xb_h.at[:, cols], xb.at[:, cols], sems.at[len(pairs) + nb])

    def start(*cs):
        for c in cs:
            c.start()

    def wait(*cs):
        for c in cs:
            c.wait()

    start(*c_slab[0], *c_slab[1])
    for t in range(NT):
        qa[t, D:D + 8, :] = zero
        vtb[t, D:D + 8, :] = zero
        qb[t, D // 2:D // 2 + 8, :] = jnp.zeros((8, T), u32)
    for t in range(QT):
        ktb[t, D // 2:D // 2 + 8, :] = jnp.zeros((8, T), u32)

    def put_qa(nb, y):
        for t in range(QT):
            qa[nb * QT + t, 0:D, :] = _tile(y, t) * QSCALE

    def qa_proj(nb):
        put_qa(nb, _dot(_unpack(wta[...]), xa[:, blk(nb)]))

    y = None
    for k, ready, queued in zip(slabs, c_slab, (c_slab[2], [c_xa1], [c_xa2, c_xa3, c_wka, c_wva, c_wqkv])):
        wait(*ready)
        start(*queued)
        w = wqa[k, :].T
        wta[:, k] = _pack(w)
        part = _dot(w, xa[k, blk(0)])
        y = part if y is None else y + part
    put_qa(0, y)
    wait(c_xa1)
    qa_proj(1)
    wait(c_xa2, c_xa3, c_wka, c_wva)
    start(c_xb(0))
    pad = jnp.zeros((HR - DH, D), f32)
    wkv = jnp.concatenate([wka[...].astype(f32), pad, wva[...].astype(f32), pad], axis=0).astype(bf16)
    kv = _round(_dot(wkv, xa[...]))
    last = _iota((8, S), 0) == DH - 16
    vta[0:16, :] = kv[HR:HR + 16]
    vta[16:HR, :] = jnp.where(last, 1.0, kv[HR + 16:])
    kt = kv[0:HR]
    kmax = _round(jnp.sqrt(jnp.max(jnp.sum(kt * kt, axis=0, keepdims=True), axis=1, keepdims=True)) * SLACK)
    kt = jnp.concatenate([kt[0:16], jnp.where(last, kmax, kt[16:HR]), jnp.zeros((T - HR, S), f32)], axis=0)
    kn = kt.astype(bf16).T
    ka[...] = _pack(kn)
    for c in range(NT):
        for n, off, end in ((NVS[c], voff[c], (c + 1) * T - NFS[c]), (NFS[c], nv + foff[c], (c + 1) * T)):
            for r in range(0, n, 16):
                kk = kn[end - n + r:end - n + r + 16].astype(f32)
                for d in range(DH):
                    kbc[(off + r) // 16, d] = jnp.broadcast_to(kk[:, d:d + 1], (16, T)).reshape(2, 8, T)
    qa_proj(2)
    wait(c_wqkv)
    start(*[c_xb(nb) for nb in range(1, NB)], c_wob, c_woa)
    wtb[...] = _pack(wqkv[...].T)
    qa_proj(3)


    def b_proj(nb, _):
        wait(c_xb(nb))
        x = xb[:, dblk(nb * NQ, NQ)]
        dst = qbc.at[pl.ds(SKEW + nb * H * QR * QT, H * QR * QT)]

        def q_rows():
            for h in range(H):
                for t in range(QT):
                    tok = yield
                    q = qa[nb * QT + t, h * DH:h * DH + HR, :]
                    q = [after(q[r:r + 8], tok, 2 + r // 8) for r in range(0, HR, 8)]
                    q[2] = jnp.where(row < DH - 16, q[2], 0.0)
                    nrm = jnp.sum(q[0] * q[0] + q[1] * q[1] + q[2] * q[2], axis=0, keepdims=True)
                    q[2] = jnp.where(row == DH - 16, nrm * lax.rsqrt(nrm + 1e-30) * -SLACK, q[2])
                    w = packed(jnp.concatenate(q + [zero], axis=0), D)
                    for i in range(2):
                        dst[(h * QR + DH + 1 + i) * QT + t] = pltpu.bitcast(w[8 * i:8 * i + 8], f32)
                    q = _unpack(w).astype(f32)
                    q = [q[r:r + 8] for r in range(0, HR, 8)]
                    for d in [DH] + list(range(DH)):
                        if d % 4 == 0:
                            tok = yield
                            q[d // 8] = after(q[d // 8], tok, 2)
                        qd = jnp.broadcast_to(q[d // 8][d % 8:d % 8 + 1], (8, T))
                        if d == DH:
                            qd = qd * kmax
                            s = qd
                        else:
                            s = s + kbc[nv // 16, d] * qd
                        dst[(h * QR + d) * QT + t] = qd
                    pf[nb * H + h, :, t * T:(t + 1) * T] = packed(jnp.exp2(s).reshape(nf, T), D + 16)

        def k_tiles():
            for g in range(H // HPT):
                for t in range(QT):
                    tok = yield
                    parts = []
                    for h in range(g * HPT, (g + 1) * HPT):
                        k = ktb[t, h * DH // 2:h * DH // 2 + 16, :]
                        parts += [k[0:8], jnp.where(row == 0, k[8:16], jnp.uint32(0))]
                    parts[0] = _pack(after(pltpu.bitcast(parts[0], f32), tok, 1))
                    kn = _pack(_unpack(jnp.concatenate(parts, axis=0)).T)
                    kb[g, nb * QT + t] = kn
                    kr[g, nb * QT + t] = pltpu.roll(kn, 32, 1)
                    side.done(pltpu.bitcast(kn[T // 2 - 8:], f32))

        side.add(q_rows(), H * QT * 6, 3 * PG, 18)
        for r0 in range(0, D, MC):
            k = packed(proj(wtb, D + r0, D + r0 + MC, x), r0 // 2)
            for t in range(QT):
                ktb[t, r0 // 2:(r0 + MC) // 2, :] = _tile(k, t)
        side.add(k_tiles(), H // HPT * QT, 3 * PG // 2)
        for r0 in range(0, D, MC):
            q = packed(proj(wtb, r0, r0 + MC, x) * QSCALE, (D + r0) // 2)
            for t in range(QT):
                qb[nb * QT + t, r0 // 2:(r0 + MC) // 2, :] = _tile(q, t)
        for r0 in range(0, D, MC):
            v = _round(proj(wtb, 2 * D + r0, 2 * D + r0 + MC, x))
            for t in range(QT):
                vtb[nb * QT + t, r0:r0 + MC, :] = _tile(v, t)
        side.flush()

    lax.fori_loop(0, NB, b_proj, None)

    upper = _iota((T, T), 0) > _iota((T, T), 1)
    r, c = 2 * _iota((T // 2, T), 0), _iota((T // 2, T), 1)
    umask[...] = (jnp.where(r > c, jnp.uint32(0xFFFF), jnp.uint32(0))
                  | jnp.where(r >= c, jnp.uint32(0xFFFF0000), jnp.uint32(0)))

    def b_scores(g, t):
        lane = _iota((16, T), 1)
        q = []
        for j in range(HPT):
            qj = qb[t, pl.ds((g * HPT + j) * (DH // 2), 16), :]
            q.append(jnp.concatenate([qj[0:8], jnp.where(row == 0, qj[8:16], jnp.uint32(0))], axis=0))

        def scores(k, js, split=None):
            cols = []
            for j in js:
                w = [jnp.zeros((16, T), u32)] * HPT
                if split is None:
                    w[j] = q[j]
                else:
                    w[j] = jnp.where(lane < split, q[j], jnp.uint32(0))
                    w[(j + 1) % HPT] = q[j] ^ w[j]
                cols.append(jnp.concatenate(w, axis=0))
            s = _dot(_unpack(k), _unpack(jnp.concatenate(cols, axis=1)))
            return [_tile(s, i) for i in range(len(js))]

        if t >= 2:
            fold = [[] for _ in range(HPT)]
            even = (_iota((BU // 2, T), 1) & 32) == 0
            for r in range(0, T - BU, BU):
                old = kb[g, t - 2, r // 2:(r + BU) // 2, :]
                new = kr[g, t, (r + BU) // 2:(r + 2 * BU) // 2, :]
                for js, k in (([0, 2], jnp.where(even, old, new)), ([1, 3], jnp.where(even, new, old))):
                    for j, x in zip(js, scores(k, js, r + BU)):
                        fold[j].append(x)
            rest = scores(jnp.concatenate([kb[g, t - 2, (T - BU) // 2:T // 2, :], kb[g, t - 1],
                                           kb[g, t, 0:BU // 2, :]], axis=0), range(HPT))
            s = []
            for j in range(HPT):
                oldest = jnp.concatenate(fold[j] + [rest[j][0:BU]], axis=0)
                newest = jnp.concatenate([rest[j][BU + T:]] + fold[j], axis=0)
                s.append(jnp.concatenate([jnp.where(upper, oldest, newest), rest[j][BU:BU + T]], axis=0))
        elif t == 1:
            s = [jnp.concatenate([jnp.where(upper, NEG, x[T:]), x[0:T]], axis=0)
                 for x in scores(jnp.concatenate([kb[g, 0], kb[g, 1]], axis=0), range(HPT))]
        else:
            s = [jnp.where(upper, NEG, x) for x in scores(kb[g, 0], range(HPT))]
        for j in range(HPT):
            n = s[j].shape[0]
            sb[t, 0:n, j * T:(j + 1) * T] = s[j]
            m = jnp.max(s[j].reshape(n // 8, 8, T), axis=0)
            mb[t, :, j * T:(j + 1) * T] = jnp.broadcast_to(jnp.max(m, axis=0, keepdims=True), (8, T))

    def b_pv(g, t):
        n = 2 * T if t >= 1 else T
        p = packed(jnp.exp2(sb[t, 0:n, :].reshape(n // 8, 8, HPT * T) - mb[t]).reshape(n, HPT * T), t * T)
        if t >= 2:
            oldest = p[0:T // 2] & jnp.concatenate([umask[...]] * HPT, axis=1)
            p = jnp.concatenate([oldest, p[T // 2:], p[0:T // 2] ^ oldest], axis=0)
        elif t == 1:
            p = jnp.concatenate([p[T // 2:], p[0:T // 2]], axis=0)
        for j in range(HPT):
            h = g * HPT + j
            v = []
            for c in range(max(0, t - 2), t + 1):
                vc = vtb[c, pl.ds(h * DH, HR), :]
                v.append(jnp.concatenate([vc[0:16], jnp.where(row == DH - 16, 1.0, vc[16:HR])], axis=0))
            put_head(t, h, _dot(jnp.concatenate(v, axis=1), _unpack(_tile(p, j))))

    def b_step(g, _):
        for t in range(NT):
            b_pv(g, t)
            b_scores(g + 1, t)

    wait(c_wob, c_woa)
    wtob[...] = _pack(wob[...].T)
    wtoa[...] = _pack(woa[...].T)
    for t in range(NT):
        b_scores(0, t)
    lax.fori_loop(0, H // HPT - 1, b_step, None)

    def q_row(ref, j, d):
        return ref[(j * QR + d) * QT:(j * QR + d + 1) * QT]

    def vpu_probs(qref, every):
        for j in range(JA):
            for g in range(nv // 16):
                for d in range(DH):
                    tok = yield
                    if d == 0:
                        s = jnp.broadcast_to(q_row(qref, j, DH), (2, QT, 8, T))
                    if d % every == 0:
                        s = after(s, tok, 5)
                    s = s + kbc[g, d][:, None] * q_row(qref, j, d)
                e = jnp.exp2(jnp.concatenate([_untile(s[0]), _untile(s[1])], axis=0))
                pv.at[j][8 * g:8 * g + 8, :] = _pack(e.astype(bf16))

    def a_weights(qref, j):
        return _pack(jnp.concatenate([_untile(q_row(qref, j, DH + i)) for i in (1, 2)], axis=0))

    def p_rows(c):
        r0 = c * T - voff[c] - foff[c]
        return slice(r0 // 2, (r0 + T - NVS[c] - NFS[c]) // 2)

    def a_probs(w, j, c):
        k = paced(ka[c * T // 2:((c + 1) * T - NVS[c] - NFS[c]) // 2, :])
        e = jnp.exp2(_dot(_unpack(k)[:, 0:32], _unpack(w)))
        pa.at[j][p_rows(c), :] = _pack(e.astype(bf16))
        side.rows(e)

    def a_pv(u, j, c, acc):
        p = [pa[j, p_rows(c), :], pv[j, voff[c] // 2:voff[c + 1] // 2, :]]
        if NFS[c]:
            p.append(pf[u])
        r = _dot(vta[:, c * T:(c + 1) * T], _unpack(jnp.concatenate(p, axis=0)))
        return r if acc is None else acc + r

    def a_done(u, acc, low):
        nb = lax.shift_right_logical(u, H.bit_length() - 1)
        for t in range(QT):
            put_head(nb * QT + t, u & (H - 1), _tile(acc, t))
            low = jnp.minimum(low, _tile(acc[16:HR], t))
        return low

    def heads_out(nb):
        return jnp.concatenate([ot[nb * QT + t] for t in range(QT)], axis=1).astype(bf16)

    def out_copy(rows, c0, c1, sem):
        return pltpu.make_async_copy(outv.at[rows, c0:c1], out_h.at[rows, c0:c1], osems.at[sem])

    groups = JA * (S - nv - nf) // 16
    steps = JA * DH * (nv // 16)
    split = D + 64
    b_copy = out_copy(slice(0, S), split, 2 * D, NB)

    qref = qbc.at[pl.ds(SKEW, JA * QR * QT)]
    side.add(vpu_probs(qref, 2), steps, groups + NB * PG, 16)
    for nb in range(NB + 1):
        if nb < NB:
            for n in range(JA // NB * NT):
                j, c = nb * JA // NB + n // NT, n % NT
                a_probs(a_weights(qref, j), j, c)
                if n % 8 == 4:
                    b_pv(H // HPT - 1, nb * QT + n // 8)
        if nb > 0:
            o = heads_out(nb - 1)
            for c0 in range(D - T, 0, -T):
                write_out(proj(wtob, c0, c0 + T, o), (nb - 1) * NQ, D + c0)
            obt[:, blk(nb - 1)] = proj(wtob, 0, split - D, o)
    side.flush()
    start(b_copy)

    def a_step(i, carry):
        base, low = carry
        qref = qbc.at[pl.ds(base, JA * QR * QT)]
        side.add(vpu_probs(qref, 3), steps, groups, 16)
        for j in range(JA):
            w, acc = a_weights(qref, j), None
            for c in range(NT):
                acc = a_pv(i * JA + j, j, c, acc)
                a_probs(w, j, c)
            low = a_done(i * JA + j, acc, low)
        side.flush()
        return base + JA * QR * QT, low

    _, low = lax.fori_loop(0, NU // JA - 1, a_step, (jnp.int32(SKEW + JA * QR * QT), jnp.ones((8, T), f32)))

    def last_pv():
        nonlocal low
        for j in range(JA):
            acc = None
            for c in range(NT):
                yield
                acc = a_pv(NU - JA + j, j, c, acc)
            low = a_done(jnp.int32(NU - JA + j), acc, low)

    def a_out(nb, between=None):
        o = heads_out(nb)
        for c0 in range(0, D, T):
            y = proj(wtoa, c0, min(c0 + T, D), o, between)
            if c0 + T > D:
                y = jnp.concatenate([y, obt[:, blk(nb) if isinstance(nb, int) else dblk(nb * NQ, NQ)]], axis=0)
            write_out(y, nb * NQ, c0)

    tail = _spread(last_pv(), JA * NT, EARLY * (-(-D // T)) ** 2)
    for nb in range(EARLY):
        a_out(nb, tail)
    side.flush()
    start(*[out_copy(blk(nb), 0, split, nb) for nb in range(EARLY)])
    unsafe = jnp.logical_not(jnp.min(jnp.where(row == DH - 16, low, 1.0)) >= L_MIN)

    @pl.when(unsafe)
    def _():
        def exact(u, _):
            w = a_weights(qbc.at[pl.ds(SKEW + u * QR * QT, QR * QT)], 0)
            w = jnp.where(_iota((16, NQ), 0) < DH // 2, w, jnp.uint32(0))
            s = _dot(_unpack(ka[...])[:, 0:32], _unpack(w))
            p = jnp.exp2(s - jnp.max(s, axis=0, keepdims=True)).astype(bf16)
            a_done(u, _dot(vta[...], p), zero)

        lax.fori_loop(0, NU, exact, None)
        wait(*[out_copy(blk(nb), 0, split, nb) for nb in range(EARLY)])

    def finish(nb, _):
        a_out(nb)
        side.flush()
        start(out_copy(dblk(nb * NQ, NQ), 0, split, nb))

    lax.fori_loop(jnp.where(unsafe, 0, EARLY), NB, finish, None)
    wait(*[out_copy(blk(nb), 0, split, nb) for nb in range(NB)], b_copy)


@jax.jit
def pallas_concat_heads__grouped_kv_mqa__sliding_block__prompt_kernel(
    A_x: jax.Array,
    A_wq: jax.Array,
    A_wk: jax.Array,
    A_wv: jax.Array,
    A_wo: jax.Array,
    B_x: jax.Array,
    B_wqkv: jax.Array,
    B_wo: jax.Array,
):
    vmem = pltpu.VMEM
    hbm = pl.BlockSpec(memory_space=pltpu.HBM)
    nv, nf = sum(NVS), sum(NFS)
    out = pl.pallas_call(
        _kernel,
        out_shape=jax.ShapeDtypeStruct((S, 2 * D), bf16),
        in_specs=[hbm] * 8,
        out_specs=hbm,
        scratch_shapes=[
            vmem((D, S), bf16), vmem((D, S), bf16),
            vmem((D, D), bf16), vmem((DH, D), bf16),
            vmem((DH, D), bf16), vmem((D, D), bf16),
            vmem((D, 3 * D), bf16), vmem((D, D), bf16),
            vmem((D // 2, D), u32), vmem((3 * D // 2, D), u32),
            vmem((D // 2, D), u32), vmem((D // 2, D), u32),
            vmem((NT, D + 8, T), f32),
            vmem((S // 2, T), u32),
            vmem((HR, S), f32),
            vmem(((nv + nf) // 16, DH, 2, 8, T), f32),
            vmem((NU * QR * QT + 4, 8, T), f32),
            vmem((JA, (S - nv - nf) // 2, NQ), u32),
            vmem((JA, nv // 2, NQ), u32),
            vmem((NU, nf // 2, NQ), u32),
            vmem((NT, D // 2 + 8, T), u32),
            vmem((QT, D // 2 + 8, T), u32),
            vmem((H // HPT, NT, T // 2, T), u32),
            vmem((H // HPT, NT, T // 2, T), u32),
            vmem((NT, D + 8, T), f32),
            vmem((NT, 2 * T, HPT * T), f32),
            vmem((NT, 8, HPT * T), f32),
            vmem((T // 2, T), u32),
            vmem((NT, D, T), f32),
            vmem((64, S), f32),
            vmem((S, 2 * D), bf16),
            vmem((7, QT, 8, T), f32),
            vmem((S, NQ), u32),
            pltpu.SemaphoreType.DMA((2 * len(KS) + 6 + NB,)),
            pltpu.SemaphoreType.DMA((NB + 1,)),
        ],
        compiler_params=pltpu.CompilerParams(vmem_limit_bytes=126 * 2 ** 20),
        name="attn_pair",
    )(A_x.reshape(S, D).T, A_wq, A_wk.T, A_wv.T, A_wo, B_x.reshape(S, D).T, B_wqkv, B_wo)
    return out.reshape(1, S, 2 * D)
```

```python
import jax
import jax.numpy as jnp
import numpy as np
from jax import lax
import jax.experimental.pallas as pl
import jax.experimental.pallas.tpu as pltpu

f32, bf16, u32, i32 = jnp.float32, jnp.bfloat16, jnp.uint32, jnp.int32

S = 2048
D = 576
H = 32
DH = 18
T = 128
NT = S // T
QT = 4
NQ = QT * T
NB = S // NQ
NU = NB * H
HR = 24
HPT = 4
BU = 32
QSCALE = float(DH ** -0.5 * np.log2(np.e))
SLACK = 1.02
HEADROOM = 64.0
L_MIN = float(2.0 ** -50)
NEG = -1e30

JA = 8
NVS = [32, 16, 16] * 5 + [16]
NFS = [0] * 15 + [16]
QR = DH + 3
SKEW = 1
QA = D + 8
GR = HPT * DH
MC = 96
KS = [0, 128, 256, D]
EARLY = 2
PG = -(-D // T) * D // 16
LEAD = 40


def _dot(a, b):
    return lax.dot_general(a, b, (((1,), (0,)), ((), ())), preferred_element_type=f32)


def _pack(x):
    return pltpu.bitcast(x, u32)


def _unpack(x):
    return pltpu.bitcast(x, bf16)


def _round(x):
    return x.astype(bf16).astype(f32)


def _iota(shape, axis):
    return lax.broadcasted_iota(i32, shape, axis)


def _tile(y, t):
    return y[:, t * T:(t + 1) * T]


def _untile(y):
    return jnp.concatenate([y[t] for t in range(QT)], axis=1)


class _Side:
    def __init__(self):
        self.jobs, self.due, self.clock, self.token = [], [], 0, None

    def add(self, gen, steps, ticks, ahead=0):
        next(gen)
        self.jobs.append(dict(gen=gen, steps=steps, ticks=ticks, ahead=ahead, done=0, seen=0))

    def _run(self, job, upto):
        while job["done"] < min(job["steps"], upto):
            try:
                job["gen"].send(self.token if job["done"] >= job["ahead"] else jnp.zeros((8, T), f32))
            except StopIteration:
                pass
            job["done"] += 1

    def rows(self, y):
        for r in range(0, y.shape[0], 16):
            self.clock += 1
            self.token = y[r + 8:r + 16, y.shape[1] - T:]
            for job in self.jobs:
                job["seen"] += 1
                self._run(job, job["ahead"] - (-job["seen"] * job["steps"] // job["ticks"]))

    def done(self, val):
        self.due.append((self.clock + LEAD, val))

    def take(self):
        ready = [v for t, v in self.due if t <= self.clock]
        self.due = [(t, v) for t, v in self.due if t > self.clock]
        return ready

    def flush(self):
        for job in self.jobs:
            self._run(job, job["steps"])
        self.jobs, self.due = [], []


def _spread(gen, steps, calls):
    next(gen)
    counts = iter([(n + 1) * steps // calls - n * steps // calls for n in range(calls)])

    def call():
        for _ in range(next(counts)):
            next(gen, None)

    return call


def _kernel(xa_h, wqa_h, wka_h, wva_h, woa_h, xb_h, wqkv_h, wob_h, out_h,
            xa, xb, wqa, wka, wva, woa, wqkv, wob, wta, wtb, wtoa, wtob,
            qa, ka, vta, kbc, qbc, pa, pv, pf,
            qb, ktb, kb, kr, vtb, sb, mb, umask,
            ot, obt, outv, order, tmp, sems, osems):
    voff = [int(x) for x in np.cumsum([0] + NVS)]
    foff = [int(x) for x in np.cumsum([0] + NFS)]
    nv, nf = voff[-1], foff[-1]
    row = _iota((8, T), 0)
    zero = jnp.zeros((8, T), f32)
    side = _Side()

    def blk(nb):
        return slice(nb * NQ, (nb + 1) * NQ)

    def dblk(start, size):
        return pl.ds(pl.multiple_of(start, size), size)

    def group(ref, g, t, rows):
        return ref.at[pl.ds(8 * SKEW + (g * NT + t) * rows, rows)]

    def views(*bases):
        n = (48, T // 2, T // 2, GR + 8)
        return [ref.at[pl.ds(base * 8, NT * rows)]
                for ref, base, rows in zip((qb, kb, kr, vtb), (bases[0], bases[1], bases[1], bases[2]), n)]

    def after(val, tok, i):
        at = (slice(i, i + val.shape[0]), slice(0, val.shape[1])) if val.ndim == 4 else (i, 0)
        order[at] = jnp.broadcast_to(tok, val.shape)
        order[at] = val
        return order[at]

    def paced(lhs):
        ready = side.take()
        if not ready:
            return lhs
        top = pltpu.bitcast(lhs[0:8], f32)
        for tok in ready:
            top = after(top, tok, 0)
        return jnp.concatenate([_pack(top), lhs[8:]], axis=0)

    def packed(e, r0):
        at = (slice(r0, r0 + e.shape[0] // 2), slice(0, e.shape[1]))
        tmp[at] = _pack(e.astype(bf16))
        return tmp[at]

    def proj(w_ref, r0, r1, x, between=None):
        y = None
        for k0 in range(0, D, T):
            k1 = min(k0 + T, D)
            if between is not None:
                between()
            w = w_ref[r0 // 2:r1 // 2, k0:k1]
            part = _dot(_unpack(paced(w) if k1 - k0 == T else w), x[k0:k1])
            side.rows(part)
            y = part if y is None else y + part
        return y

    def write_out(y, r0, c0):
        def tiles():
            for t in range(QT):
                tok = yield
                yt = _tile(y, t)
                yt = jnp.concatenate([after(yt[0:8], tok, 1), yt[8:]], axis=0).astype(bf16).T
                r = r0 + t * T
                outv[slice(r, r + T) if isinstance(r, int) else dblk(r, T), c0:c0 + T] = yt
                side.done(yt[T - 16:T].astype(f32)[8:16])

        side.add(tiles(), QT, 20)

    def put_head(t, h, o):
        den = o[DH:DH + 1]
        inv = pl.reciprocal(den, approx=True)
        ot[t, pl.ds(h * DH, DH), :] = (o * (inv * (2.0 - den * inv)))[0:DH]

    slabs = [slice(a, b) for a, b in zip(KS[:-1], KS[1:])]
    pairs = [(src.at[k, cols], dst.at[k, cols]) for k in slabs
             for src, dst, cols in ((wqa_h, wqa, slice(None)), (xa_h, xa, blk(0)))]
    pairs += [(xa_h.at[:, blk(nb)], xa.at[:, blk(nb)]) for nb in range(1, NB)]
    pairs += [(wka_h, wka), (wva_h, wva), (wqkv_h, wqkv), (wob_h, wob), (woa_h, woa)]
    copies = [pltpu.make_async_copy(src, dst, sems.at[n]) for n, (src, dst) in enumerate(pairs)]
    c_slab = [copies[2 * n:2 * n + 2] for n in range(len(slabs))]
    c_xa1, c_xa2, c_xa3, c_wka, c_wva, c_wqkv, c_wob, c_woa = copies[2 * len(slabs):]

    def c_xb(nb):
        cols = blk(nb) if isinstance(nb, int) else dblk(nb * NQ, NQ)
        return pltpu.make_async_copy(xb_h.at[:, cols], xb.at[:, cols], sems.at[len(pairs) + nb])

    def start(*cs):
        for c in cs:
            c.start()

    def wait(*cs):
        for c in cs:
            c.wait()

    start(*c_slab[0], *c_slab[1])
    for t in range(NT):
        qa[8 * SKEW + t * QA + D:8 * SKEW + (t + 1) * QA, :] = zero
    for t in range(QT):
        ktb[t, D // 2:D // 2 + 8, :] = jnp.zeros((8, T), u32)

    def put_qa(nb, y):
        for t in range(QT):
            r0 = 8 * SKEW + (nb * QT + t) * QA
            qa[r0:r0 + D, :] = _tile(y, t) * QSCALE

    def qa_proj(nb):
        put_qa(nb, _dot(_unpack(wta[...]), xa[:, blk(nb)]))

    y = None
    for k, ready, queued in zip(slabs, c_slab, (c_slab[2], [c_xa1], [c_xa2, c_xa3, c_wka, c_wva, c_wqkv])):
        wait(*ready)
        start(*queued)
        w = wqa[k, :].T
        wta[:, k] = _pack(w)
        part = _dot(w, xa[k, blk(0)])
        y = part if y is None else y + part
    put_qa(0, y)
    wait(c_xa1)
    qa_proj(1)
    wait(c_xa2, c_xa3, c_wka, c_wva)
    start(c_xb(0))
    pad = jnp.zeros((HR - DH, D), f32)
    wkv = jnp.concatenate([wka[...].astype(f32), pad, wva[...].astype(f32), pad], axis=0).astype(bf16)
    kv = _round(_dot(wkv, xa[...]))
    last = _iota((8, S), 0) == DH - 16
    vta[0:16, :] = kv[HR:HR + 16]
    vta[16:HR, :] = jnp.where(last, 1.0, kv[HR + 16:])
    kt = kv[0:HR]
    kmax = _round(jnp.sqrt(jnp.max(jnp.sum(kt * kt, axis=0, keepdims=True), axis=1, keepdims=True)) * SLACK)
    hi = jnp.where(last, kmax, jnp.where(_iota((8, S), 0) == DH - 15, 1.0, kt[16:HR]))
    kt = jnp.concatenate([kt[0:16], hi, jnp.zeros((T - HR, S), f32)], axis=0)
    kn = kt.astype(bf16).T
    ka[...] = _pack(kn)
    for c in range(NT):
        for n, off, end in ((NVS[c], voff[c], (c + 1) * T - NFS[c]), (NFS[c], nv + foff[c], (c + 1) * T)):
            for r in range(0, n, 16):
                kk = kn[end - n + r:end - n + r + 16].astype(f32)
                for d in range(DH):
                    kbc[(off + r) // 16, d] = jnp.broadcast_to(kk[:, d:d + 1], (16, T)).reshape(2, 8, T)
    qa_proj(2)
    wait(c_wqkv)
    start(*[c_xb(nb) for nb in range(1, NB)], c_wob, c_woa)
    wtb[...] = _pack(wqkv[...].T)
    qa_proj(3)


    def b_proj(nb, base):
        src = qa.at[pl.ds(base * 8, QT * QA)]
        wait(c_xb(nb))
        x = xb[:, dblk(nb * NQ, NQ)]
        dst = qbc.at[pl.ds(SKEW + nb * H * QR * QT, H * QR * QT)]

        def q_rows():
            for h in range(H):
                for t in range(QT):
                    tok = yield
                    q = src[t * QA + h * DH:t * QA + h * DH + HR, :]
                    q = [after(q[r:r + 8], tok, 2 + r // 8) for r in range(0, HR, 8)]
                    q[2] = jnp.where(row < DH - 16, q[2], 0.0)
                    nrm = jnp.sum(q[0] * q[0] + q[1] * q[1] + q[2] * q[2], axis=0, keepdims=True)
                    q[2] = jnp.where(row == DH - 16, nrm * lax.rsqrt(nrm + 1e-30) * -SLACK,
                                     jnp.where(row == DH - 15, HEADROOM, q[2]))
                    w = packed(jnp.concatenate(q + [zero], axis=0), D)
                    for i in range(2):
                        dst[(h * QR + DH + 1 + i) * QT + t] = pltpu.bitcast(w[8 * i:8 * i + 8], f32)
                    q = _unpack(w).astype(f32)
                    q = [q[r:r + 8] for r in range(0, HR, 8)]
                    for d in [DH] + list(range(DH)):
                        if d % 4 == 0:
                            tok = yield
                            q[d // 8] = after(q[d // 8], tok, 2)
                        qd = jnp.broadcast_to(q[d // 8][d % 8:d % 8 + 1], (8, T))
                        if d == DH:
                            qd = qd * kmax + HEADROOM
                            s = qd
                        else:
                            s = s + kbc[nv // 16, d] * qd
                        dst[(h * QR + d) * QT + t] = qd
                    pf[nb * H + h, :, t * T:(t + 1) * T] = packed(jnp.exp2(s).reshape(nf, T), D + 16)

        def k_tiles():
            for g in range(H // HPT):
                for t in range(QT):
                    tok = yield
                    parts = []
                    for h in range(g * HPT, (g + 1) * HPT):
                        k = ktb[t, h * DH // 2:h * DH // 2 + 16, :]
                        parts += [k[0:8], jnp.where(row == 0, k[8:16], jnp.uint32(0))]
                    parts[0] = _pack(after(pltpu.bitcast(parts[0], f32), tok, 1))
                    kn = _pack(_unpack(jnp.concatenate(parts, axis=0)).T)
                    group(kb, g, nb * QT + t, T // 2)[...] = kn
                    group(kr, g, nb * QT + t, T // 2)[...] = pltpu.roll(kn, 32, 1)
                    side.done(pltpu.bitcast(kn[T // 2 - 8:], f32))

        def put_groups(ref, y, r0, size, rows):
            for t in range(QT):
                for g in range(r0 // size, -(-(r0 + y.shape[0]) // size)):
                    a, b = max(r0, g * size), min(r0 + y.shape[0], (g + 1) * size)
                    at = group(ref, g, nb * QT + t, rows)
                    at[a - g * size:b - g * size, :] = _tile(y[a - r0:b - r0], t)
                    if b == (g + 1) * size:
                        at[size:rows, :] = jnp.zeros((rows - size, T), y.dtype)

        side.add(q_rows(), H * QT * 6, 3 * PG, 18)
        for r0 in range(0, D, MC):
            k = packed(proj(wtb, D + r0, D + r0 + MC, x), r0 // 2)
            for t in range(QT):
                ktb[t, r0 // 2:(r0 + MC) // 2, :] = _tile(k, t)
        side.add(k_tiles(), H // HPT * QT, 3 * PG // 2)
        for r0 in range(0, D, MC):
            q = packed(proj(wtb, r0, r0 + MC, x) * QSCALE, (D + r0) // 2)
            put_groups(qb, q, r0 // 2, GR // 2, 48)
        for r0 in range(0, D, MC):
            v = _round(proj(wtb, 2 * D + r0, 2 * D + r0 + MC, x))
            put_groups(vtb, v, r0, GR, GR + 8)
        side.flush()
        return base + QT * QA // 8

    lax.fori_loop(0, NB, b_proj, jnp.int32(SKEW))

    upper = _iota((T, T), 0) > _iota((T, T), 1)
    r, c = 2 * _iota((T // 2, T), 0), _iota((T // 2, T), 1)
    umask[...] = (jnp.where(r > c, jnp.uint32(0xFFFF), jnp.uint32(0))
                  | jnp.where(r >= c, jnp.uint32(0xFFFF0000), jnp.uint32(0)))

    def b_scores(qg, kg, rg, t):
        lane = _iota((16, T), 1)
        q = []
        for j in range(HPT):
            qj = qg[t * 48 + j * DH // 2:t * 48 + j * DH // 2 + 16, :]
            q.append(jnp.concatenate([qj[0:8], jnp.where(row == 0, qj[8:16], jnp.uint32(0))], axis=0))

        def scores(k, js, split=None):
            cols = []
            for j in js:
                w = [jnp.zeros((16, T), u32)] * HPT
                if split is None:
                    w[j] = q[j]
                else:
                    w[j] = jnp.where(lane < split, q[j], jnp.uint32(0))
                    w[(j + 1) % HPT] = q[j] ^ w[j]
                cols.append(jnp.concatenate(w, axis=0))
            s = _dot(_unpack(k), _unpack(jnp.concatenate(cols, axis=1)))
            return [_tile(s, i) for i in range(len(js))]

        if t >= 2:
            fold = [[] for _ in range(HPT)]
            even = (_iota((BU // 2, T), 1) & 32) == 0
            for r in range(0, T - BU, BU):
                old = kg[((t - 2) * T + r) // 2:((t - 2) * T + r + BU) // 2, :]
                new = rg[(t * T + r + BU) // 2:(t * T + r + 2 * BU) // 2, :]
                for js, k in (([0, 2], jnp.where(even, old, new)), ([1, 3], jnp.where(even, new, old))):
                    for j, x in zip(js, scores(k, js, r + BU)):
                        fold[j].append(x)
            rest = scores(kg[((t - 1) * T - BU) // 2:(t * T + BU) // 2, :], range(HPT))
            s = []
            for j in range(HPT):
                oldest = jnp.concatenate(fold[j] + [rest[j][0:BU]], axis=0)
                newest = jnp.concatenate([rest[j][BU + T:]] + fold[j], axis=0)
                s.append(jnp.concatenate([jnp.where(upper, oldest, newest), rest[j][BU:BU + T]], axis=0))
        elif t == 1:
            s = [jnp.concatenate([jnp.where(upper, NEG, x[T:]), x[0:T]], axis=0)
                 for x in scores(kg[0:T, :], range(HPT))]
        else:
            s = [jnp.where(upper, NEG, x) for x in scores(kg[0:T // 2, :], range(HPT))]
        for j in range(HPT):
            n = s[j].shape[0]
            sb[t, 0:n, j * T:(j + 1) * T] = s[j]
            m = jnp.max(s[j].reshape(n // 8, 8, T), axis=0)
            mb[t, :, j * T:(j + 1) * T] = jnp.broadcast_to(jnp.max(m, axis=0, keepdims=True), (8, T))

    def b_pv(g, vg, t):
        n = 2 * T if t >= 1 else T
        p = packed(jnp.exp2(sb[t, 0:n, :].reshape(n // 8, 8, HPT * T) - mb[t]).reshape(n, HPT * T), t * T)
        if t >= 2:
            oldest = p[0:T // 2] & jnp.concatenate([umask[...]] * HPT, axis=1)
            p = jnp.concatenate([oldest, p[T // 2:], p[0:T // 2] ^ oldest], axis=0)
        elif t == 1:
            p = jnp.concatenate([p[T // 2:], p[0:T // 2]], axis=0)
        for j in range(HPT):
            h = g * HPT + j
            v = []
            for c in range(max(0, t - 2), t + 1):
                vc = vg[c * (GR + 8) + j * DH:c * (GR + 8) + j * DH + HR, :]
                v.append(jnp.concatenate([vc[0:16], jnp.where(row == DH - 16, 1.0, vc[16:HR])], axis=0))
            put_head(t, h, _dot(jnp.concatenate(v, axis=1), _unpack(_tile(p, j))))

    strides = (NT * 48 // 8, NT * T // 16, NT * (GR + 8) // 8)

    def b_step(g, bases):
        qg, kg, rg, vg = views(*bases)
        for t in range(NT):
            b_pv(g, vg, t)
            b_scores(qg, kg, rg, t)
        return tuple(b + n for b, n in zip(bases, strides))

    wait(c_wob, c_woa)
    wtob[...] = _pack(wob[...].T)
    wtoa[...] = _pack(woa[...].T)
    for t in range(NT):
        b_scores(*views(SKEW, SKEW, SKEW)[0:3], t)
    lax.fori_loop(0, H // HPT - 1, b_step,
                  (jnp.int32(SKEW + strides[0]), jnp.int32(SKEW + strides[1]), jnp.int32(SKEW)))

    def q_row(ref, j, d):
        return ref[(j * QR + d) * QT:(j * QR + d + 1) * QT]

    def vpu_probs(qref, every):
        for j in range(JA):
            for g in range(nv // 16):
                for d in range(DH):
                    tok = yield
                    if d == 0:
                        s = jnp.broadcast_to(q_row(qref, j, DH), (2, QT, 8, T))
                    if d % every == 0:
                        s = after(s, tok, 5)
                    s = s + kbc[g, d][:, None] * q_row(qref, j, d)
                e = jnp.exp2(jnp.concatenate([_untile(s[0]), _untile(s[1])], axis=0))
                pv.at[j][8 * g:8 * g + 8, :] = _pack(e.astype(bf16))

    def a_weights(qref, j):
        return _pack(jnp.concatenate([_untile(q_row(qref, j, DH + i)) for i in (1, 2)], axis=0))

    def p_rows(c):
        r0 = c * T - voff[c] - foff[c]
        return slice(r0 // 2, (r0 + T - NVS[c] - NFS[c]) // 2)

    def a_probs(w, j, c):
        k = paced(ka[c * T // 2:((c + 1) * T - NVS[c] - NFS[c]) // 2, :])
        e = jnp.exp2(_dot(_unpack(k)[:, 0:32], _unpack(w)))
        pa.at[j][p_rows(c), :] = _pack(e.astype(bf16))
        side.rows(e)

    def a_pv(u, j, c, acc):
        p = [pa[j, p_rows(c), :], pv[j, voff[c] // 2:voff[c + 1] // 2, :]]
        if NFS[c]:
            p.append(pf[u])
        r = _dot(vta[:, c * T:(c + 1) * T], _unpack(jnp.concatenate(p, axis=0)))
        return r if acc is None else acc + r

    def a_done(u, acc, low):
        nb = lax.shift_right_logical(u, H.bit_length() - 1)
        for t in range(QT):
            put_head(nb * QT + t, u & (H - 1), _tile(acc, t))
            low = jnp.minimum(low, _tile(acc[16:HR], t))
        return low

    def heads_out(nb):
        return jnp.concatenate([ot[nb * QT + t] for t in range(QT)], axis=1).astype(bf16)

    def out_copy(rows, c0, c1, sem):
        return pltpu.make_async_copy(outv.at[rows, c0:c1], out_h.at[rows, c0:c1], osems.at[sem])

    groups = JA * (S - nv - nf) // 16
    steps = JA * DH * (nv // 16)
    split = D + 64
    b_copy = out_copy(slice(0, S), split, 2 * D, NB)

    qref = qbc.at[pl.ds(SKEW, JA * QR * QT)]
    side.add(vpu_probs(qref, 2), steps, groups + NB * PG, 16)
    for nb in range(NB + 1):
        if nb < NB:
            for n in range(JA // NB * NT):
                j, c = nb * JA // NB + n // NT, n % NT
                a_probs(a_weights(qref, j), j, c)
                if n % 8 == 4:
                    b_pv(H // HPT - 1, views(0, 0, SKEW + (H // HPT - 1) * strides[2])[3], nb * QT + n // 8)
        if nb > 0:
            o = heads_out(nb - 1)
            for c0 in range(D - T, 0, -T):
                write_out(proj(wtob, c0, c0 + T, o), (nb - 1) * NQ, D + c0)
            obt[:, blk(nb - 1)] = proj(wtob, 0, split - D, o)
    side.flush()
    start(b_copy)

    def a_step(i, carry):
        base, low = carry
        qref = qbc.at[pl.ds(base, JA * QR * QT)]
        side.add(vpu_probs(qref, 3), steps, groups, 16)
        for j in range(JA):
            w, acc = a_weights(qref, j), None
            for c in range(NT):
                acc = a_pv(i * JA + j, j, c, acc)
                a_probs(w, j, c)
            low = a_done(i * JA + j, acc, low)
        side.flush()
        return base + JA * QR * QT, low

    _, low = lax.fori_loop(0, NU // JA - 1, a_step, (jnp.int32(SKEW + JA * QR * QT), jnp.ones((8, T), f32)))

    def last_pv():
        nonlocal low
        for j in range(JA):
            acc = None
            for c in range(NT):
                yield
                acc = a_pv(NU - JA + j, j, c, acc)
            low = a_done(jnp.int32(NU - JA + j), acc, low)

    def a_out(nb, between=None):
        o = heads_out(nb)
        for c0 in range(0, D, T):
            y = proj(wtoa, c0, min(c0 + T, D), o, between)
            if c0 + T > D:
                y = jnp.concatenate([y, obt[:, blk(nb) if isinstance(nb, int) else dblk(nb * NQ, NQ)]], axis=0)
            write_out(y, nb * NQ, c0)

    tail = _spread(last_pv(), JA * NT, EARLY * (-(-D // T)) ** 2)
    for nb in range(EARLY):
        a_out(nb, tail)
    side.flush()
    start(*[out_copy(blk(nb), 0, split, nb) for nb in range(EARLY)])
    unsafe = jnp.logical_not(jnp.min(jnp.where(row == DH - 16, low, 1.0)) >= L_MIN)

    @pl.when(unsafe)
    def _():
        def exact(u, _):
            w = a_weights(qbc.at[pl.ds(SKEW + u * QR * QT, QR * QT)], 0)
            w = jnp.where(_iota((16, NQ), 0) < DH // 2, w, jnp.uint32(0))
            s = _dot(_unpack(ka[...])[:, 0:32], _unpack(w))
            p = jnp.exp2(s - jnp.max(s, axis=0, keepdims=True)).astype(bf16)
            a_done(u, _dot(vta[...], p), zero)

        lax.fori_loop(0, NU, exact, None)
        wait(*[out_copy(blk(nb), 0, split, nb) for nb in range(EARLY)])

    def finish(nb, _):
        a_out(nb)
        side.flush()
        start(out_copy(dblk(nb * NQ, NQ), 0, split, nb))

    lax.fori_loop(jnp.where(unsafe, 0, EARLY), NB, finish, None)
    wait(*[out_copy(blk(nb), 0, split, nb) for nb in range(NB)], b_copy)


@jax.jit
def pallas_concat_heads__grouped_kv_mqa__sliding_block__prompt_kernel(
    A_x: jax.Array,
    A_wq: jax.Array,
    A_wk: jax.Array,
    A_wv: jax.Array,
    A_wo: jax.Array,
    B_x: jax.Array,
    B_wqkv: jax.Array,
    B_wo: jax.Array,
):
    vmem = pltpu.VMEM
    hbm = pl.BlockSpec(memory_space=pltpu.HBM)
    nv, nf = sum(NVS), sum(NFS)
    out = pl.pallas_call(
        _kernel,
        out_shape=jax.ShapeDtypeStruct((S, 2 * D), bf16),
        in_specs=[hbm] * 8,
        out_specs=hbm,
        scratch_shapes=[
            vmem((D, S), bf16), vmem((D, S), bf16),
            vmem((D, D), bf16), vmem((DH, D), bf16),
            vmem((DH, D), bf16), vmem((D, D), bf16),
            vmem((D, 3 * D), bf16), vmem((D, D), bf16),
            vmem((D // 2, D), u32), vmem((3 * D // 2, D), u32),
            vmem((D // 2, D), u32), vmem((D // 2, D), u32),
            vmem((NT * QA + 32, T), f32),
            vmem((S // 2, T), u32),
            vmem((HR, S), f32),
            vmem(((nv + nf) // 16, DH, 2, 8, T), f32),
            vmem((NU * QR * QT + 4, 8, T), f32),
            vmem((JA, (S - nv - nf) // 2, NQ), u32),
            vmem((JA, nv // 2, NQ), u32),
            vmem((NU, nf // 2, NQ), u32),
            vmem((H // HPT * NT * 48 + 32, T), u32),
            vmem((QT, D // 2 + 8, T), u32),
            vmem((H // HPT * S // 2 + 32, T), u32),
            vmem((H // HPT * S // 2 + 32, T), u32),
            vmem((H // HPT * NT * (GR + 8) + 32, T), f32),
            vmem((NT, 2 * T, HPT * T), f32),
            vmem((NT, 8, HPT * T), f32),
            vmem((T // 2, T), u32),
            vmem((NT, D, T), f32),
            vmem((64, S), f32),
            vmem((S, 2 * D), bf16),
            vmem((7, QT, 8, T), f32),
            vmem((S, NQ), u32),
            pltpu.SemaphoreType.DMA((2 * len(KS) + 6 + NB,)),
            pltpu.SemaphoreType.DMA((NB + 1,)),
        ],
        compiler_params=pltpu.CompilerParams(vmem_limit_bytes=126 * 2 ** 20),
        name="attn_pair",
    )(A_x.reshape(S, D).T, A_wq, A_wk.T, A_wv.T, A_wo, B_x.reshape(S, D).T, B_wqkv, B_wo)
    return out.reshape(1, S, 2 * D)
```

```python
import jax
import jax.numpy as jnp
import numpy as np
from jax import lax
import jax.experimental.pallas as pl
import jax.experimental.pallas.tpu as pltpu

f32, bf16, u32, i32 = jnp.float32, jnp.bfloat16, jnp.uint32, jnp.int32

S = 2048
D = 576
H = 32
DH = 18
T = 128
NT = S // T
QT = 4
NQ = QT * T
NB = S // NQ
NU = NB * H
HR = 24
HPT = 4
BU = 32
QSCALE = float(DH ** -0.5 * np.log2(np.e))
SLACK = 1.02
TINY = 1e-30
HEADROOM = 64.0
L_MIN = float(2.0 ** -50)
NEG = -1e30

JA = 8
NVS = [32, 16, 16] * 5 + [16]
NFS = [0] * 14 + [16] * 2
QR = DH + 3
SKEW = 1
QA = D + 8
GR = HPT * DH
MC = 96
KS = [0, 128, 256, D]
EARLY = 2
PG = -(-D // T) * D // 16
LEAD = 40


def _dot(a, b):
    return lax.dot_general(a, b, (((1,), (0,)), ((), ())), preferred_element_type=f32)


def _pack(x):
    return pltpu.bitcast(x, u32)


def _unpack(x):
    return pltpu.bitcast(x, bf16)


def _round(x):
    return x.astype(bf16).astype(f32)


def _iota(shape, axis):
    return lax.broadcasted_iota(i32, shape, axis)


def _tile(y, t):
    return y[:, t * T:(t + 1) * T]


def _untile(y):
    return jnp.concatenate([y[t] for t in range(QT)], axis=1)


class _Side:
    def __init__(self):
        self.jobs, self.due, self.clock, self.token = [], [], 0, None

    def add(self, gen, steps, ticks, ahead=0):
        next(gen)
        self.jobs.append(dict(gen=gen, steps=steps, ticks=ticks, ahead=ahead, done=0, seen=0))

    def _run(self, job, upto):
        while job["done"] < min(job["steps"], upto):
            try:
                job["gen"].send(self.token if job["done"] >= job["ahead"] else jnp.zeros((8, T), f32))
            except StopIteration:
                pass
            job["done"] += 1

    def rows(self, y):
        for r in range(0, y.shape[0], 16):
            self.clock += 1
            self.token = y[r + 8:r + 16, y.shape[1] - T:]
            for job in self.jobs:
                job["seen"] += 1
                self._run(job, job["ahead"] - (-job["seen"] * job["steps"] // job["ticks"]))

    def done(self, val):
        self.due.append((self.clock + LEAD, val))

    def take(self):
        ready = [v for t, v in self.due if t <= self.clock]
        self.due = [(t, v) for t, v in self.due if t > self.clock]
        return ready

    def flush(self):
        for job in self.jobs:
            self._run(job, job["steps"])
        self.jobs, self.due = [], []


def _spread(gen, steps, calls):
    next(gen)
    counts = iter([(n + 1) * steps // calls - n * steps // calls for n in range(calls)])

    def call():
        for _ in range(next(counts)):
            next(gen, None)

    return call


def _kernel(xa_h, wqa_h, wka_h, wva_h, woa_h, xb_h, wqkv_h, wob_h, out_h,
            xa, xb, wqa, wka, wva, woa, wqkv, wob, wta, wtb, wtoa, wtob,
            qa, ka, vta, kbc, qbc, pa, pv, pf,
            qb, ktb, kb, kr, vtb, sb, mb, umask,
            ot, obt, outv, order, tmp, sems, osems):
    voff = [int(x) for x in np.cumsum([0] + NVS)]
    foff = [int(x) for x in np.cumsum([0] + NFS)]
    nv, nf = voff[-1], foff[-1]
    row = _iota((8, T), 0)
    zero = jnp.zeros((8, T), f32)
    side = _Side()

    def blk(nb):
        return slice(nb * NQ, (nb + 1) * NQ)

    def dblk(start, size):
        return pl.ds(pl.multiple_of(start, size), size)

    def group(ref, g, t, rows):
        return ref.at[pl.ds(8 * SKEW + (g * NT + t) * rows, rows)]

    def views(*bases):
        n = (48, T // 2, T // 2, GR + 8)
        return [ref.at[pl.ds(base * 8, NT * rows)]
                for ref, base, rows in zip((qb, kb, kr, vtb), (bases[0], bases[1], bases[1], bases[2]), n)]

    def after(val, tok, i):
        at = (slice(i, i + val.shape[0]), slice(0, val.shape[1])) if val.ndim == 4 else (i, 0)
        order[at] = jnp.broadcast_to(tok, val.shape)
        order[at] = val
        return order[at]

    def paced(lhs):
        ready = side.take()
        if not ready:
            return lhs
        top = pltpu.bitcast(lhs[0:8], f32)
        for tok in ready:
            top = after(top, tok, 0)
        return jnp.concatenate([_pack(top), lhs[8:]], axis=0)

    def packed(e, r0):
        at = (slice(r0, r0 + e.shape[0] // 2), slice(0, e.shape[1]))
        tmp[at] = _pack(e.astype(bf16))
        return tmp[at]

    def proj(w_ref, r0, r1, x, between=None):
        y = None
        for k0 in range(0, D, T):
            k1 = min(k0 + T, D)
            if between is not None:
                between()
            w = w_ref[r0 // 2:r1 // 2, k0:k1]
            part = _dot(_unpack(paced(w) if k1 - k0 == T else w), x[k0 // T])
            side.rows(part)
            y = part if y is None else y + part
        return y

    def write_out(y, r0, c0):
        def tiles():
            for t in range(QT):
                tok = yield
                yt = _tile(y, t)
                yt = jnp.concatenate([after(yt[0:8], tok, 1), yt[8:]], axis=0).astype(bf16).T
                r = r0 + t * T
                outv[slice(r, r + T) if isinstance(r, int) else dblk(r, T), c0:c0 + T] = yt
                side.done(yt[T - 16:T].astype(f32)[8:16])

        side.add(tiles(), QT, 20)

    def put_head(t, h, o):
        den = o[DH:DH + 1]
        inv = pl.reciprocal(den, approx=True)
        ot[t, pl.ds(h * DH, DH), :] = (o * (inv * (2.0 - den * inv)))[0:DH]

    slabs = [slice(a, b) for a, b in zip(KS[:-1], KS[1:])]
    pairs = [(src.at[k, cols], dst.at[k, cols]) for k in slabs
             for src, dst, cols in ((wqa_h, wqa, slice(None)), (xa_h, xa, blk(0)))]
    pairs += [(xa_h.at[:, blk(nb)], xa.at[:, blk(nb)]) for nb in range(1, NB)]
    pairs += [(wka_h, wka), (wva_h, wva), (wqkv_h, wqkv), (wob_h, wob), (woa_h, woa)]
    copies = [pltpu.make_async_copy(src, dst, sems.at[n]) for n, (src, dst) in enumerate(pairs)]
    c_slab = [copies[2 * n:2 * n + 2] for n in range(len(slabs))]
    c_xa1, c_xa2, c_xa3, c_wka, c_wva, c_wqkv, c_wob, c_woa = copies[2 * len(slabs):]

    def c_xb(nb):
        cols = blk(nb) if isinstance(nb, int) else dblk(nb * NQ, NQ)
        return pltpu.make_async_copy(xb_h.at[:, cols], xb.at[:, cols], sems.at[len(pairs) + nb])

    def start(*cs):
        for c in cs:
            c.start()

    def wait(*cs):
        for c in cs:
            c.wait()

    start(*c_slab[0], *c_slab[1])
    for t in range(NT):
        qa[8 * SKEW + t * QA + D:8 * SKEW + (t + 1) * QA, :] = zero
    for t in range(QT):
        ktb[t, D // 2:D // 2 + 8, :] = jnp.zeros((8, T), u32)

    def put_qa(nb, y):
        for t in range(QT):
            r0 = 8 * SKEW + (nb * QT + t) * QA
            qa[r0:r0 + D, :] = _tile(y, t) * QSCALE

    def qa_proj(nb):
        put_qa(nb, _dot(_unpack(wta[...]), xa[:, blk(nb)]))

    y = None
    for k, ready, queued in zip(slabs, c_slab, (c_slab[2], [c_xa1], [c_xa2, c_xa3, c_wka, c_wva, c_wqkv])):
        wait(*ready)
        start(*queued)
        w = wqa[k, :].T
        wta[:, k] = _pack(w)
        part = _dot(w, xa[k, blk(0)])
        y = part if y is None else y + part
    put_qa(0, y)
    wait(c_xa1)
    qa_proj(1)
    wait(c_xa2, c_xa3, c_wka, c_wva)
    start(c_xb(0))
    pad = jnp.zeros((HR - DH, D), f32)
    wkv = jnp.concatenate([wka[...].astype(f32), pad, wva[...].astype(f32), pad], axis=0).astype(bf16)
    kv = _round(_dot(wkv, xa[...]))
    last = _iota((8, S), 0) == DH - 16
    vta[0:16, :] = kv[HR:HR + 16]
    vta[16:HR, :] = jnp.where(last, 1.0, kv[HR + 16:])
    kt = kv[0:HR]
    kmax = jnp.max(jnp.sum(kt * kt, axis=0, keepdims=True), axis=1, keepdims=True)
    kmax = _round(jnp.sqrt(kmax + TINY) * SLACK)
    hi = jnp.where(last, kmax, jnp.where(_iota((8, S), 0) == DH - 15, 1.0, kt[16:HR]))
    kt = jnp.concatenate([kt[0:16], hi, jnp.zeros((T - HR, S), f32)], axis=0)
    kn = kt.astype(bf16).T
    ka[...] = _pack(kn)
    for c in range(NT):
        for n, off, end in ((NVS[c], voff[c], (c + 1) * T - NFS[c]), (NFS[c], nv + foff[c], (c + 1) * T)):
            for r in range(0, n, 16):
                kk = kn[end - n + r:end - n + r + 16].astype(f32)
                for d in range(DH):
                    kbc[(off + r) // 16, d] = jnp.broadcast_to(kk[:, d:d + 1], (16, T)).reshape(2, 8, T)
    qa_proj(2)
    wait(c_wqkv)
    start(*[c_xb(nb) for nb in range(1, NB)], c_wob, c_woa)
    wtb[...] = _pack(wqkv[...].T)
    qa_proj(3)

    def b_proj(nb, base):
        src = qa.at[pl.ds(base * 8, QT * QA)]
        wait(c_xb(nb))
        x = [xb[k0:min(k0 + T, D), dblk(nb * NQ, NQ)] for k0 in range(0, D, T)]
        dst = qbc.at[pl.ds(SKEW + nb * H * QR * QT, H * QR * QT)]

        def q_rows():
            for h in range(H):
                for t in range(QT):
                    tok = yield
                    q = src[t * QA + h * DH:t * QA + h * DH + HR, :]
                    q = [after(q[r:r + 8], tok, 2 + r // 8) for r in range(0, HR, 8)]
                    q[2] = jnp.where(row < DH - 16, q[2], 0.0)
                    nrm = jnp.sum(q[0] * q[0] + q[1] * q[1] + q[2] * q[2], axis=0, keepdims=True) + TINY
                    q[2] = jnp.where(row == DH - 16, nrm * lax.rsqrt(nrm) * -SLACK,
                                     jnp.where(row == DH - 15, HEADROOM, q[2]))
                    w = packed(jnp.concatenate(q + [zero], axis=0), D)
                    for i in range(2):
                        dst[(h * QR + DH + 1 + i) * QT + t] = pltpu.bitcast(w[8 * i:8 * i + 8], f32)
                    q = _unpack(w).astype(f32)
                    q = [q[r:r + 8] for r in range(0, HR, 8)]
                    for d in [DH] + list(range(DH)):
                        if d % 4 == 0:
                            tok = yield
                            q[d // 8] = after(q[d // 8], tok, 2)
                        qd = jnp.broadcast_to(q[d // 8][d % 8:d % 8 + 1], (8, T))
                        if d == DH:
                            qd = qd * kmax + HEADROOM
                            s = qd
                        else:
                            s = s + kbc[nv // 16, d] * qd
                        dst[(h * QR + d) * QT + t] = qd
                    pf[nb * H + h, 0:8, t * T:(t + 1) * T] = packed(jnp.exp2(s).reshape(16, T), D + 16)

        def k_tiles():
            for g in range(H // HPT):
                for t in range(QT):
                    tok = yield
                    parts = []
                    for h in range(g * HPT, (g + 1) * HPT):
                        k = ktb[t, h * DH // 2:h * DH // 2 + 16, :]
                        parts += [k[0:8], jnp.where(row == 0, k[8:16], jnp.uint32(0))]
                    parts[0] = _pack(after(pltpu.bitcast(parts[0], f32), tok, 1))
                    kn = _pack(_unpack(jnp.concatenate(parts, axis=0)).T)
                    group(kb, g, nb * QT + t, T // 2)[...] = kn
                    group(kr, g, nb * QT + t, T // 2)[...] = pltpu.roll(kn, 32, 1)
                    side.done(pltpu.bitcast(kn[T // 2 - 8:], f32))

        def put_groups(ref, y, r0, size, rows):
            for t in range(QT):
                for g in range(r0 // size, -(-(r0 + y.shape[0]) // size)):
                    a, b = max(r0, g * size), min(r0 + y.shape[0], (g + 1) * size)
                    at = group(ref, g, nb * QT + t, rows)
                    at[a - g * size:b - g * size, :] = _tile(y[a - r0:b - r0], t)
                    if b == (g + 1) * size:
                        at[size:rows, :] = jnp.zeros((rows - size, T), y.dtype)

        side.add(q_rows(), H * QT * 6, 3 * PG, 18)
        for r0 in range(0, D, MC):
            k = packed(proj(wtb, D + r0, D + r0 + MC, x), r0 // 2)
            for t in range(QT):
                ktb[t, r0 // 2:(r0 + MC) // 2, :] = _tile(k, t)
        side.add(k_tiles(), H // HPT * QT, 3 * PG // 2)
        for r0 in range(0, D, MC):
            q = packed(proj(wtb, r0, r0 + MC, x) * QSCALE, (D + r0) // 2)
            put_groups(qb, q, r0 // 2, GR // 2, 48)
        for r0 in range(0, D, MC):
            v = _round(proj(wtb, 2 * D + r0, 2 * D + r0 + MC, x))
            put_groups(vtb, v, r0, GR, GR + 8)
        side.flush()
        return base + QT * QA // 8

    lax.fori_loop(0, NB, b_proj, jnp.int32(SKEW))

    upper = _iota((T, T), 0) > _iota((T, T), 1)
    r, c = 2 * _iota((T // 2, T), 0), _iota((T // 2, T), 1)
    umask[...] = (jnp.where(r > c, jnp.uint32(0xFFFF), jnp.uint32(0))
                  | jnp.where(r >= c, jnp.uint32(0xFFFF0000), jnp.uint32(0)))

    def b_scores(qg, kg, rg, t):
        lane = _iota((16, T), 1)
        q = []
        for j in range(HPT):
            qj = qg[t * 48 + j * DH // 2:t * 48 + j * DH // 2 + 16, :]
            q.append(jnp.concatenate([qj[0:8], jnp.where(row == 0, qj[8:16], jnp.uint32(0))], axis=0))

        def scores(k, js, split=None):
            cols = []
            for j in js:
                w = [jnp.zeros((16, T), u32)] * HPT
                if split is None:
                    w[j] = q[j]
                else:
                    w[j] = jnp.where(lane < split, q[j], jnp.uint32(0))
                    w[(j + 1) % HPT] = q[j] ^ w[j]
                cols.append(jnp.concatenate(w, axis=0))
            s = _dot(_unpack(k), _unpack(jnp.concatenate(cols, axis=1)))
            if js[0] == 0:
                side.rows(s)
            return [_tile(s, i) for i in range(len(js))]

        if t >= 2:
            fold = [[] for _ in range(HPT)]
            even = (_iota((BU // 2, T), 1) & 32) == 0
            for r in range(0, T - BU, BU):
                old = kg[((t - 2) * T + r) // 2:((t - 2) * T + r + BU) // 2, :]
                new = rg[(t * T + r + BU) // 2:(t * T + r + 2 * BU) // 2, :]
                for js, k in (([0, 2], jnp.where(even, old, new)), ([1, 3], jnp.where(even, new, old))):
                    for j, x in zip(js, scores(k, js, r + BU)):
                        fold[j].append(x)
            rest = scores(kg[((t - 1) * T - BU) // 2:(t * T + BU) // 2, :], range(HPT))
            s = []
            for j in range(HPT):
                oldest = jnp.concatenate(fold[j] + [rest[j][0:BU]], axis=0)
                newest = jnp.concatenate([rest[j][BU + T:]] + fold[j], axis=0)
                s.append(jnp.concatenate([jnp.where(upper, oldest, newest), rest[j][BU:BU + T]], axis=0))
        elif t == 1:
            s = [jnp.concatenate([jnp.where(upper, NEG, x[T:]), x[0:T]], axis=0)
                 for x in scores(kg[0:T, :], range(HPT))]
        else:
            s = [jnp.where(upper, NEG, x) for x in scores(kg[0:T // 2, :], range(HPT))]
        for j in range(HPT):
            n = s[j].shape[0]
            sb[t, 0:n, j * T:(j + 1) * T] = s[j]
            m = jnp.max(s[j].reshape(n // 8, 8, T), axis=0)
            mb[t, :, j * T:(j + 1) * T] = jnp.broadcast_to(jnp.max(m, axis=0, keepdims=True), (8, T))

    def b_pv(g, vg, t, j0=0, nh=HPT, first=None):
        n, cols = 2 * T if t >= 1 else T, slice(j0 * T, (j0 + nh) * T)
        p = packed(jnp.exp2(sb[t, 0:n, cols].reshape(n // 8, 8, nh * T) - mb[t, :, cols]).reshape(n, nh * T), t * T)
        if first is not None:
            first()
        if t >= 2:
            oldest = p[0:T // 2] & jnp.concatenate([umask[...]] * nh, axis=1)
            p = jnp.concatenate([oldest, p[T // 2:], p[0:T // 2] ^ oldest], axis=0)
        elif t == 1:
            p = jnp.concatenate([p[T // 2:], p[0:T // 2]], axis=0)
        for j in range(j0, j0 + nh):
            v = []
            for c in range(max(0, t - 2), t + 1):
                vc = vg[c * (GR + 8) + j * DH:c * (GR + 8) + j * DH + HR, :]
                v.append(jnp.concatenate([vc[0:16], jnp.where(row == DH - 16, 1.0, vc[16:HR])], axis=0))
            put_head(t, g * HPT + j, _dot(jnp.concatenate(v, axis=1), _unpack(_tile(p, j - j0))))

    def q_row(ref, j, d):
        return ref[(j * QR + d) * QT:(j * QR + d + 1) * QT]

    def vpu_probs(qref, every, store, units=JA, gs=range(nv // 16)):
        for j in range(units):
            for g in gs:
                for d in range(DH):
                    tok = yield
                    if d == 0:
                        s = jnp.broadcast_to(q_row(qref, j, DH), (2, QT, 8, T))
                    if d % every == 0:
                        s = after(s, tok, 5)
                    s = s + kbc[g, d][:, None] * q_row(qref, j, d)
                e = jnp.exp2(jnp.concatenate([_untile(s[0]), _untile(s[1])], axis=0))
                store(j, g, _pack(e.astype(bf16)))

    fu = NU // (H // HPT)

    def b_fill(g, base):
        def store(j, _, p):
            pf.at[g * fu + j][8:16, :] = p

        side.add(vpu_probs(qbc.at[pl.ds(base, fu * QR * QT)], 1, store, fu, [nv // 16 + 1]),
                 fu * DH, (NT - 2) * (2 * T + BU) // 16 + 3 * T // 16, 8)

    strides = (NT * 48 // 8, NT * T // 16, NT * (GR + 8) // 8, fu * QR * QT)

    def b_step(g, bases):
        qg, kg, rg, vg = views(*bases)
        b_fill(g + 1, bases[3])
        for t in reversed(range(NT)):
            b_pv(g, vg, t, first=lambda: b_scores(qg, kg, rg, t))
        side.flush()
        return tuple(b + n for b, n in zip(bases, strides))

    wait(c_wob, c_woa)
    wtob[...] = _pack(wob[...].T)
    wtoa[...] = _pack(woa[...].T)
    b_fill(0, SKEW)
    for t in range(NT):
        b_scores(*views(SKEW, SKEW, SKEW)[0:3], t)
    side.flush()
    lax.fori_loop(0, H // HPT - 1, b_step,
                  (jnp.int32(SKEW + strides[0]), jnp.int32(SKEW + strides[1]), jnp.int32(SKEW),
                   jnp.int32(SKEW + strides[3])))

    def keep(j, g, p):
        pv.at[j][8 * g:8 * g + 8, :] = p

    def a_weights(qref, j):
        return _pack(jnp.concatenate([_untile(q_row(qref, j, DH + i)) for i in (1, 2)], axis=0))

    def p_rows(c):
        r0 = c * T - voff[c] - foff[c]
        return slice(r0 // 2, (r0 + T - NVS[c] - NFS[c]) // 2)

    def a_probs(w, j, c):
        k = paced(ka[c * T // 2:((c + 1) * T - NVS[c] - NFS[c]) // 2, :])
        e = jnp.exp2(_dot(_unpack(k)[:, 0:32], _unpack(w)))
        pa.at[j][p_rows(c), :] = _pack(e.astype(bf16))
        side.rows(e)

    def a_pv(u, j, c, acc):
        p = [pa[j, p_rows(c), :], pv[j, voff[c] // 2:voff[c + 1] // 2, :]]
        if NFS[c]:
            p.append(pf[u, foff[c] // 2:foff[c + 1] // 2, :])
        r = _dot(vta[:, c * T:(c + 1) * T], _unpack(jnp.concatenate(p, axis=0)))
        return r if acc is None else acc + r

    def a_done(u, acc, low):
        nb = lax.shift_right_logical(u, H.bit_length() - 1)
        for t in range(QT):
            put_head(nb * QT + t, u & (H - 1), _tile(acc, t))
            low = jnp.minimum(low, _tile(acc[16:HR], t))
        return low

    def heads_out(nb):
        return [jnp.concatenate([ot[nb * QT + t, k0:min(k0 + T, D), :] for t in range(QT)], axis=1).astype(bf16)
                for k0 in range(0, D, T)]

    def out_copy(rows, c0, c1, sem):
        return pltpu.make_async_copy(outv.at[rows, c0:c1], out_h.at[rows, c0:c1], osems.at[sem])

    groups = JA * (S - nv - nf) // 16
    steps = JA * DH * (nv // 16)
    split = D + 64
    b_copy = out_copy(slice(0, S), split, 2 * D, NB)

    qref = qbc.at[pl.ds(SKEW, JA * QR * QT)]
    vg = views(0, 0, SKEW + (H // HPT - 1) * strides[2])[3]
    side.add(vpu_probs(qref, 2, keep), steps, groups + NB * PG, 16)
    for nb in range(NB + 1):
        if nb < NB:
            for n in range(JA // NB * NT):
                j, c = nb * JA // NB + n // NT, n % NT
                a_probs(a_weights(qref, j), j, c)
                if n % 2 == 0:
                    b_pv(H // HPT - 1, vg, nb * QT + n // 8, n % 8 // 2, 1)
        if nb > 0:
            o = heads_out(nb - 1)
            for c0 in range(D - T, 0, -T):
                write_out(proj(wtob, c0, c0 + T, o), (nb - 1) * NQ, D + c0)
            obt[:, blk(nb - 1)] = proj(wtob, 0, split - D, o)
    side.flush()
    start(b_copy)

    def a_step(i, carry):
        base, low = carry
        qref = qbc.at[pl.ds(base, JA * QR * QT)]
        side.add(vpu_probs(qref, 3, keep), steps, groups, 16)
        for j in range(JA):
            w, acc = a_weights(qref, j), None
            for c in range(NT):
                acc = a_pv(i * JA + j, j, c, acc)
                a_probs(w, j, c)
            low = a_done(i * JA + j, acc, low)
        side.flush()
        return base + JA * QR * QT, low

    _, low = lax.fori_loop(0, NU // JA - 1, a_step, (jnp.int32(SKEW + JA * QR * QT), jnp.ones((8, T), f32)))

    def last_pv():
        nonlocal low
        for j in range(JA):
            acc = None
            for c in range(NT):
                yield
                acc = a_pv(NU - JA + j, j, c, acc)
            low = a_done(jnp.int32(NU - JA + j), acc, low)

    def a_out(nb, between=None):
        o = heads_out(nb)
        for c0 in range(0, D, T):
            y = proj(wtoa, c0, min(c0 + T, D), o, between)
            if c0 + T > D:
                y = jnp.concatenate([y, obt[:, blk(nb) if isinstance(nb, int) else dblk(nb * NQ, NQ)]], axis=0)
            write_out(y, nb * NQ, c0)

    tail = _spread(last_pv(), JA * NT, EARLY * (-(-D // T)) ** 2)
    for nb in range(EARLY):
        a_out(nb, tail)
    side.flush()
    start(*[out_copy(blk(nb), 0, split, nb) for nb in range(EARLY)])
    unsafe = jnp.logical_not(jnp.min(jnp.where(row == DH - 16, low, 1.0)) >= L_MIN)

    @pl.when(unsafe)
    def _():
        def exact(n, _):
            u, t = lax.shift_right_logical(n, QT.bit_length() - 1), n & (QT - 1)
            at = SKEW + (u * QR + DH + 1) * QT + t
            w = _pack(jnp.concatenate([qbc[at], qbc[at + QT]], axis=0))
            w = jnp.where(_iota((16, T), 0) < DH // 2, w, jnp.uint32(0))
            s = _dot(_unpack(ka[...])[:, 0:32], _unpack(w))
            p = jnp.exp2(s - jnp.max(s, axis=0, keepdims=True)).astype(bf16)
            put_head(lax.shift_right_logical(u, H.bit_length() - 1) * QT + t, u & (H - 1), _dot(vta[...], p))

        lax.fori_loop(0, NU * QT, exact, None)
        wait(*[out_copy(blk(nb), 0, split, nb) for nb in range(EARLY)])

    def finish(nb, _):
        a_out(nb)
        side.flush()
        start(out_copy(dblk(nb * NQ, NQ), 0, split, nb))

    lax.fori_loop(jnp.where(unsafe, 0, EARLY), NB, finish, None)
    wait(*[out_copy(blk(nb), 0, split, nb) for nb in range(NB)], b_copy)


@jax.jit
def pallas_concat_heads__grouped_kv_mqa__sliding_block__prompt_kernel(
    A_x: jax.Array,
    A_wq: jax.Array,
    A_wk: jax.Array,
    A_wv: jax.Array,
    A_wo: jax.Array,
    B_x: jax.Array,
    B_wqkv: jax.Array,
    B_wo: jax.Array,
):
    vmem = pltpu.VMEM
    hbm = pl.BlockSpec(memory_space=pltpu.HBM)
    nv, nf = sum(NVS), sum(NFS)
    out = pl.pallas_call(
        _kernel,
        out_shape=jax.ShapeDtypeStruct((S, 2 * D), bf16),
        in_specs=[hbm] * 8,
        out_specs=hbm,
        scratch_shapes=[
            vmem((D, S), bf16), vmem((D, S), bf16),
            vmem((D, D), bf16), vmem((DH, D), bf16),
            vmem((DH, D), bf16), vmem((D, D), bf16),
            vmem((D, 3 * D), bf16), vmem((D, D), bf16),
            vmem((D // 2, D), u32), vmem((3 * D // 2, D), u32),
            vmem((D // 2, D), u32), vmem((D // 2, D), u32),
            vmem((NT * QA + 32, T), f32),
            vmem((S // 2, T), u32),
            vmem((HR, S), f32),
            vmem(((nv + nf) // 16, DH, 2, 8, T), f32),
            vmem((NU * QR * QT + 4, 8, T), f32),
            vmem((JA, (S - nv - nf) // 2, NQ), u32),
            vmem((JA, nv // 2, NQ), u32),
            vmem((NU, nf // 2, NQ), u32),
            vmem((H // HPT * NT * 48 + 32, T), u32),
            vmem((QT, D // 2 + 8, T), u32),
            vmem((H // HPT * S // 2 + 32, T), u32),
            vmem((H // HPT * S // 2 + 32, T), u32),
            vmem((H // HPT * NT * (GR + 8) + 32, T), f32),
            vmem((NT, 2 * T, HPT * T), f32),
            vmem((NT, 8, HPT * T), f32),
            vmem((T // 2, T), u32),
            vmem((NT, D, T), f32),
            vmem((64, S), f32),
            vmem((S, 2 * D), bf16),
            vmem((7, QT, 8, T), f32),
            vmem((S, NQ), u32),
            pltpu.SemaphoreType.DMA((2 * len(KS) + 6 + NB,)),
            pltpu.SemaphoreType.DMA((NB + 1,)),
        ],
        compiler_params=pltpu.CompilerParams(vmem_limit_bytes=126 * 2 ** 20),
        name="attn_pair",
    )(A_x.reshape(S, D).T, A_wq, A_wk.T, A_wv.T, A_wo, B_x.reshape(S, D).T, B_wqkv, B_wo)
    return out.reshape(1, S, 2 * D)
```
